```python
import os as _os
_os.environ.setdefault("JAX_PLATFORMS", "cpu")
import jax
import jax.numpy as jnp

def _softmax(x, axis=-1):
    return jax.nn.softmax(x, axis=axis)
def _gelu(x):
    return jax.nn.gelu(x, approximate=True)
def _silu(x):
    return jax.nn.silu(x)
def _sigmoid(x):
    return jax.nn.sigmoid(x)
def _layernorm(x, axis=-1, eps=1e-5):
    m = jnp.mean(x, axis=axis, keepdims=True)
    v = jnp.var(x, axis=axis, keepdims=True)
    return (x - m) / jnp.sqrt(v + eps)
def _scatter_add(tgt, idx, src, axis=0):
    return tgt.at[idx].add(src)
def _segment_sum(src, seg, n):
    return jax.ops.segment_sum(src, seg, n)
class _Rng:
    def __init__(self, key):
        self._k = key
    def _next(self):
        self._k, sub = jax.random.split(self._k)
        return sub
    def normal(self, shape):
        return jax.random.normal(self._next(), shape, dtype=jnp.bfloat16)
    def randint(self, lo, hi, shape):
        return jax.random.randint(self._next(), shape, lo, hi, dtype=jnp.int32)
    def uniform(self, shape, lo=0.0, hi=1.0):
        return jax.random.uniform(self._next(), shape, jnp.bfloat16, lo, hi)
    def permutation(self, n):
        return jax.random.permutation(self._next(), n)


kernel_name = 'sequential_preLN__softmax_full_mha__dense_activation_gelu__prompt'

def setup_inputs():
    _rng = _Rng(jax.random.key(int.from_bytes(__import__("os").urandom(4), "little")))
    _w = (lambda a: (lambda t: t.astype(jnp.bfloat16) if jnp.issubdtype(t.dtype, jnp.floating) else t)(jnp.asarray(a)))
    def _A_setup():
        B, S, D = 1, 2048, 512
        return {
            "x": _w((lambda *s: _rng.normal(s) * 0.05)(B, S, D)),
            "wqkv": _w((lambda *s: _rng.normal(s) * 0.05)(D, 3 * D)),
            "wo": _w((lambda *s: _rng.normal(s) * 0.05)(D, D)),
        }
    _A_in = _A_setup()

    def _B_setup():
        B, S, D, F = 1, 2048, 512, 1792
        return {
            "x": _w((lambda *s: _rng.normal(s) * 0.05)(B, S, D)),
            "w1": _w((lambda *s: _rng.normal(s) * 0.4)(D, F) * (D ** -0.5)),
            "b1": _w((lambda *s: _rng.normal(s) * 0.4)(F) * 0.01),
            "w2": _w((lambda *s: _rng.normal(s) * 0.4)(F, D) * (F ** -0.5)),
            "b2": _w((lambda *s: _rng.normal(s) * 0.05)(D) * 0.01),
        }
    _B_in = _B_setup()

    return {
        "A_x": _A_in["x"],
        "A_wqkv": _A_in["wqkv"],
        "A_wo": _A_in["wo"],
        "B_x": _B_in["x"],
        "B_w1": _B_in["w1"],
        "B_b1": _B_in["b1"],
        "B_w2": _B_in["w2"],
        "B_b2": _B_in["b2"],
    }

def reference(A_x, A_wqkv, A_wo, B_x, B_w1, B_b1, B_w2, B_b2):
    def _A_ref(x, wqkv, wo):
        B, S, D = x.shape
        H = 32; Dh = D // H
        qkv = (lambda x, *d: x.transpose(*d))((x @ wqkv).reshape(B, S, 3, H, Dh), 2, 0, 3, 1, 4)
        q, k, v = qkv[0], qkv[1], qkv[2]
        scale = Dh ** -0.5
        scores = jnp.einsum("bhqd,bhkd->bhqk", q, k) * scale
        p = _softmax(scores, axis=-1)
        o = jnp.einsum("bhqk,bhkd->bhqd", p, v)
        return (lambda x, *d: x.transpose(*d))(o, 0, 2, 1, 3).reshape(B, S, D) @ wo

    def _B_ref(x, w1, b1, w2, b2):
        h = jnp.einsum("bsd,df->bsf", x, w1) + b1
        h = _gelu(h)
        return jnp.einsum("bsf,fd->bsd", h, w2) + b2

    x = A_x
    h = x + _A_ref(_layernorm(x, axis=-1), A_wqkv, A_wo)
    h2 = h + _B_ref(_layernorm(h, axis=-1), B_w1, B_b1, B_w2, B_b2)
    return h2
```

```python
import functools
import math

import jax
import jax.numpy as jnp
from jax import lax
import jax.experimental.pallas as pl
import jax.experimental.pallas.tpu as pltpu

_BF = jnp.bfloat16
_F32 = jnp.float32
_U32 = jnp.uint32

H = 32
DH = 16
KC = 128
TQ = 512
HU = 4
SKEW = 18
T1 = 512
T3 = 512
FC = 256
EPS = 1e-5


def _layernorm(x):
    m = jnp.mean(x, axis=-1, keepdims=True)
    xc = x - m
    v = jnp.mean(xc * xc, axis=-1, keepdims=True)
    return xc * lax.rsqrt(v + EPS)


def _gelu(x):
    c = math.sqrt(2.0 / math.pi)
    return 0.5 * x * (1.0 + jnp.tanh(c * (x + 0.044715 * (x * x * x))))


def _kernel(x_hbm, wqkv_hbm, wo_hbm, w1_hbm, w2_hbm, b1_ref, b2_ref, out_hbm,
            x_v, wqkv_v, wo_v, w1_v, w2_v, wqvt, kh, vt, qt, ot, sbuf, obuf,
            sem_in, sem_out, *, S, D, F):
    n1 = S // T1
    n3 = S // T3
    nq = S // TQ
    nc = S // KC
    nitem = nq * H

    def x_copy(i):
        return pltpu.make_async_copy(x_hbm.at[pl.ds(i * T1, T1)], x_v.at[pl.ds(i * T1, T1)],
                                     sem_in.at[i])

    w_copies = [
        pltpu.make_async_copy(wqkv_hbm, wqkv_v, sem_in.at[n1]),
        pltpu.make_async_copy(wo_hbm, wo_v, sem_in.at[n1 + 1]),
        pltpu.make_async_copy(w1_hbm, w1_v, sem_in.at[n1 + 2]),
        pltpu.make_async_copy(w2_hbm, w2_v, sem_in.at[n1 + 3]),
    ]
    x_copy(0).start()
    w_copies[0].start()
    for i in range(1, n1):
        x_copy(i).start()
    for c in w_copies[1:]:
        c.start()

    w_copies[0].wait()
    wqvt[0:D // 2, :] = pltpu.bitcast(wqkv_v[:, 0:D].T, _U32)
    wqvt[D // 2:D, :] = pltpu.bitcast(wqkv_v[:, 2 * D:3 * D].T, _U32)
    qscale = (DH ** -0.5) * math.log2(math.e)

    def phase1(i, carry):
        x_copy(i).wait()
        r0 = pl.multiple_of(i * T1, T1)
        xn = _layernorm(x_v[pl.ds(r0, T1), :].astype(_F32)).astype(_BF)
        kf = jnp.dot(xn, wqkv_v[:, D:2 * D], preferred_element_type=_F32)
        ku = pltpu.bitcast(kf.astype(_BF), _U32)
        rh = pl.multiple_of(i * (T1 // 2), T1 // 2)
        for g in range(D // 128):
            kg = ku[:, g * 128:(g + 1) * 128]
            for j in range(128 // DH):
                kr = kg if j == 0 else pltpu.roll(kg, 128 - DH * j, axis=1)
                kh[g * (128 // DH) + j, pl.ds(rh, T1 // 2), :] = kr
        qv = lax.dot_general(pltpu.bitcast(wqvt[...], _BF), xn, (((1,), (1,)), ((), ())),
                             preferred_element_type=_F32)
        qt[i] = pltpu.bitcast((qv[0:D] * qscale).astype(_BF), _U32)
        vt[i] = pltpu.bitcast(qv[D:2 * D].astype(_BF), _U32)
        return carry

    lax.fori_loop(0, n1, phase1, 0)

    cpt = T1 // KC

    def stage_a(item, c, slot, m8):
        item = jnp.minimum(item, nitem - 1)
        h = item % H
        qi = item // H
        kc = pltpu.bitcast(kh[h, pl.ds(c * (KC // 2), KC // 2), :], _BF)[:, :DH]
        q = pltpu.bitcast(qt[qi, pl.ds(pl.multiple_of(h * (DH // 2), DH // 2), DH // 2), :], _BF)
        s = jnp.dot(kc, q, preferred_element_type=_F32)
        sbuf[slot] = s
        mc = jnp.max(s.reshape(KC // 8, 8, TQ), axis=0)
        return mc if m8 is None else jnp.maximum(m8, mc)

    def stage_p(item, c, slot, m, l8, acc):
        h = item % H
        p3 = jnp.exp2(sbuf[slot].reshape(KC // 8, 8, TQ) - m[None])
        for j in range(KC // 8 - 1, -1, -1):
            l8 = p3[j] if l8 is None else l8 + p3[j]
        v = pltpu.bitcast(
            vt[c // cpt, pl.ds(pl.multiple_of(h * (DH // 2), DH // 2), DH // 2),
               pl.ds((c % cpt) * KC, KC)], _BF)
        pv = jnp.dot(v, p3.reshape(KC, TQ).astype(_BF), preferred_element_type=_F32)
        return l8, (pv if acc is None else acc + pv)

    def finish_max(m8):
        return jnp.broadcast_to(jnp.max(m8, axis=0, keepdims=True), (8, TQ))

    m8 = None
    mcur = None
    for u in range(SKEW):
        m8 = stage_a(u // nc, u % nc, u % (2 * nc), m8)
        if u % nc == nc - 1:
            mcur = finish_max(m8)
            m8 = None

    def attn_body(i, carry):
        mcur, m8 = carry
        mnext = None
        hist = []
        l8 = acc = None
        for t in range(HU * nc):
            u = t + SKEW
            c = t % nc
            if c == 0:
                l8 = acc = None
                if t > 0:
                    mcur = mnext
            m8 = stage_a(i * HU + u // nc, u % nc, u % (2 * nc), m8)
            if u % nc == nc - 1:
                mnext = finish_max(m8)
                m8 = None
            meff = mcur
            if len(hist) >= 2:
                a = hist[-2][:8]
                meff = jnp.where(jnp.isnan(a), a, mcur)
            item = i * HU + t // nc
            l8, acc = stage_p(item, c, t % (2 * nc), meff, l8, acc)
            hist.append(acc)
            if c == nc - 1:
                h = item % H
                qi = item // H
                o = acc * (1.0 / jnp.sum(l8, axis=0, keepdims=True))
                ot[qi, pl.ds(pl.multiple_of(h * (DH // 2), DH // 2), DH // 2), :] = (
                    pltpu.bitcast(o.astype(_BF), _U32))
        return mnext, m8

    lax.fori_loop(0, nitem // HU, attn_body, (mcur, m8))

    for c in w_copies[1:]:
        c.wait()

    def out_copy(i):
        return pltpu.make_async_copy(obuf.at[pl.ds(i * T3, T3)], out_hbm.at[pl.ds(i * T3, T3)],
                                     sem_out.at[i])

    def phase3(i, carry):
        r0 = pl.multiple_of(i * T3, T3)
        o_t = pltpu.bitcast(ot[i], _BF)
        attn = lax.dot_general(o_t, wo_v[...], (((0,), (0,)), ((), ())),
                               preferred_element_type=_F32)
        hres = x_v[pl.ds(r0, T3), :].astype(_F32) + attn
        hn = _layernorm(hres).astype(_BF)
        acc = hres + b2_ref[...].astype(_F32)
        for f0 in range(0, F, FC):
            z = jnp.dot(hn, w1_v[:, f0:f0 + FC], preferred_element_type=_F32)
            z = _gelu(z + b1_ref[:, f0:f0 + FC].astype(_F32)).astype(_BF)
            acc = acc + jnp.dot(z, w2_v[f0:f0 + FC, :], preferred_element_type=_F32)
        obuf[pl.ds(r0, T3), :] = acc.astype(obuf.dtype)
        out_copy(i).start()
        return carry

    lax.fori_loop(0, n3, phase3, 0)
    for i in range(n3):
        out_copy(i).wait()


@jax.jit
def pallas_sequential_preLN__softmax_full_mha__dense_activation_gelu__prompt_kernel(
    A_x: jax.Array,
    A_wqkv: jax.Array,
    A_wo: jax.Array,
    B_x: jax.Array,
    B_w1: jax.Array,
    B_b1: jax.Array,
    B_w2: jax.Array,
    B_b2: jax.Array,
):
    B, S, D = A_x.shape
    F = B_w1.shape[1]
    assert B == 1 and D == H * DH and T1 == TQ == T3
    x = A_x.reshape(S, D)
    any_spec = pl.BlockSpec(memory_space=pl.ANY)
    vmem_spec = pl.BlockSpec(memory_space=pltpu.VMEM)
    out = pl.pallas_call(
        functools.partial(_kernel, S=S, D=D, F=F),
        out_shape=jax.ShapeDtypeStruct((S, D), A_x.dtype),
        in_specs=[any_spec] * 5 + [vmem_spec] * 2,
        out_specs=any_spec,
        scratch_shapes=[
            pltpu.VMEM((S, D), _BF),
            pltpu.VMEM((D, 3 * D), _BF),
            pltpu.VMEM((D, D), _BF),
            pltpu.VMEM((D, F), _BF),
            pltpu.VMEM((F, D), _BF),
            pltpu.VMEM((D, D), _U32),
            pltpu.VMEM((H, S // 2, 128), _U32),
            pltpu.VMEM((S // T1, D // 2, T1), _U32),
            pltpu.VMEM((S // TQ, D // 2, TQ), _U32),
            pltpu.VMEM((S // TQ, D // 2, TQ), _U32),
            pltpu.VMEM((2 * S // KC, KC, TQ), _F32),
            pltpu.VMEM((S, D), _BF),
            pltpu.SemaphoreType.DMA((S // T1 + 4,)),
            pltpu.SemaphoreType.DMA((S // T3,)),
        ],
        compiler_params=pltpu.CompilerParams(vmem_limit_bytes=100 * 1024 * 1024),
    )(x, A_wqkv, A_wo, B_w1, B_w2, B_b1.reshape(1, F), B_b2.reshape(1, D))
    return out.reshape(B, S, D)
```

```python
import functools
import math

import jax
import jax.numpy as jnp
from jax import lax
import jax.experimental.pallas as pl
import jax.experimental.pallas.tpu as pltpu

_BF = jnp.bfloat16
_F32 = jnp.float32
_U32 = jnp.uint32
_I32 = jnp.int32
_I8 = jnp.int8

H = 32
DH = 16
HG = 128 // DH
TQ = 512
FC = 256
EPS = 1e-5

KF = 256
GP = 2
NREP = 6
SA = 3
SC = 2
CMAX = 32.0
LMAX = 2.0 ** 40
KQR = 64
CARRY = 0
OSPLIT = 4
P1U = 1
BFP = 0

KC = 256
FORCE_SLOW = False


def _tie(val, dep):
    return jnp.where(dep != dep, dep, val)


def _layernorm(x, dep=None):
    r, d = x.shape
    m = jnp.broadcast_to(jnp.mean(x, axis=-1, keepdims=True), (r, 128))
    if dep is not None:
        m = _tie(m, dep)
    xc = x - jnp.concatenate([m] * (d // 128), axis=1)
    v = jnp.mean(xc * xc, axis=-1, keepdims=True)
    return xc * lax.rsqrt(v + EPS)


def _gelu(x):
    c = math.sqrt(2.0 / math.pi)
    return 0.5 * x * (1.0 + jnp.tanh(c * (x + 0.044715 * (x * x * x))))


def _rnd(x):
    return jnp.round(x).astype(_I32)


def _recip(x):
    r = pl.reciprocal(x, approx=True)
    return r * (2.0 - x * r)


def _pack8(x):
    return pltpu.bitcast(x.astype(_I8), _U32)


def _nt_dot(a, b):
    return lax.dot_general(a, b, (((1,), (1,)), ((), ())), preferred_element_type=_F32)


def _kernel(x_hbm, wqkv_hbm, wo_hbm, w1_hbm, w2_hbm, b1_hbm, b2_hbm, out_hbm,
            b1_ref, b2_ref, x_v, wqkv_v, wo_v, w1_v, w2_v, wqvt, xn_s, kf_s, cm_s, kh8, qw, sq, skb, vt, ot,
            scar, hres_s, obuf, kh, qt, sbuf, sem_in, sem_out, *, S, D, F):
    nt = S // TQ
    nsub = TQ // 128
    ng = D // 128
    qscale = (DH ** -0.5) * math.log2(math.e)

    def x_copy(i):
        return pltpu.make_async_copy(x_hbm.at[pl.ds(i * TQ, TQ)], x_v.at[pl.ds(i * TQ, TQ)],
                                     sem_in.at[i])

    def wqkv_copy(j):
        return pltpu.make_async_copy(wqkv_hbm.at[:, pl.ds(j * D, D)], wqkv_v.at[j],
                                     sem_in.at[nt + j])

    w_copies = [
        pltpu.make_async_copy(wo_hbm, wo_v, sem_in.at[nt + 3]),
        pltpu.make_async_copy(w1_hbm, w1_v, sem_in.at[nt + 4]),
        pltpu.make_async_copy(w2_hbm, w2_v, sem_in.at[nt + 5]),
        pltpu.make_async_copy(b1_hbm, b1_ref, sem_in.at[nt + 6]),
        pltpu.make_async_copy(b2_hbm, b2_ref, sem_in.at[nt + 7]),
    ]
    x_copy(0).start()
    wqkv_copy(1).start()
    for i in range(1, nt):
        x_copy(i).start()
    wqkv_copy(2).start()
    wqkv_copy(0).start()
    for c in w_copies:
        c.start()

    blk8 = lax.broadcasted_iota(_I32, (8, 128), 1) // DH
    blk = lax.broadcasted_iota(_I32, (KQR // 4, 128), 1) // DH
    odd_blk = (blk & 1) == 1
    odd_pair = (blk & 2) == 2
    hi_half = blk >= 4
    zpg = TQ // KQR
    nz = ng * zpg

    def ln1(i, n, dep):
        r0 = pl.multiple_of(i * TQ + n * 128, 128)
        xn = _layernorm(x_v[pl.ds(r0, 128), :].astype(_F32), dep).astype(_BF)
        xn_s[i, n * 64:(n + 1) * 64, :] = pltpu.bitcast(xn, _U32)

    def kdot(i, g):
        kg = jnp.dot(pltpu.bitcast(xn_s[i], _BF), wqkv_v[1, :, g * 128:(g + 1) * 128],
                     preferred_element_type=_F32)
        kf_s[i, g] = kg
        cm_s[i, g] = jnp.max(jnp.abs(kg).reshape(TQ // 8, 8, 128), axis=0)
        return kg

    def kscale(i, g):
        cm = cm_s[i, g]
        inv = None
        for j in range(HG):
            mh = jnp.max(jnp.where(blk8 == j, cm, 0.0), axis=1, keepdims=True)
            mh = jnp.maximum(jnp.max(mh, axis=0, keepdims=True), 1e-30)
            mh = jnp.broadcast_to(mh, (8, 128))
            skb[i, g * HG + j] = mh * (1.0 / (NREP * 127.0 * 127.0))
            inv = mh if inv is None else jnp.where(blk8 == j, mh, inv)
        return 127.0 * _recip(inv)

    def kq0(i, g, z, inv):
        b0 = (z * KQR) // 128 * 128
        src = b0 + 128 - (z * KQR - b0) - KQR
        w = kf_s[i, g, src:src + KQR, :].reshape(KQR // 8, 8, 128) * inv[None]
        w = jnp.concatenate([w[r] for r in range(KQR // 8 - 1, -1, -1)], axis=0)
        ci = _rnd(w)
        c = _pack8(ci)
        d = _pack8(_rnd((w - ci.astype(_F32)) * float(NREP * 2 ** SA)))
        cs = _pack8(_rnd(w * (2.0 ** -SC)))
        return (c, d, pltpu.roll(c, 16, axis=1), pltpu.roll(c, 112, axis=1),
                pltpu.roll(cs, 16, axis=1), pltpu.roll(cs, 112, axis=1))

    def kq1(st):
        c, d, cu, cd, su, sd = st
        a_e = [jnp.where(odd_blk, cu, c), jnp.where(odd_blk, c, cd)]
        e_e = [jnp.where(odd_blk, su, d), jnp.where(odd_blk, d, sd)]
        return [(a_e[e], e_e[e], pltpu.roll(a_e[e], 32, axis=1), pltpu.roll(a_e[e], 96, axis=1))
                for e in range(2)]

    def kq2(st):
        out = []
        for e in range(2):
            a, ee, up, dn = st[e]
            for f in range(2):
                if f == 0:
                    full = jnp.where(odd_pair, up, a)
                    own = jnp.where(odd_pair, up, ee)
                else:
                    full = jnp.where(odd_pair, a, dn)
                    own = jnp.where(odd_pair, ee, dn)
                out.append((2 * f + e, own, pltpu.roll(full, 64, axis=1)))
        return out

    def kq3(i, g, z, st):
        r0 = pl.multiple_of(i * (TQ // 4) + z * (KQR // 4), KQR // 4)
        for j, own, oth in st:
            kh8[g * HG + j, pl.ds(r0, KQR // 4), :] = jnp.where(hi_half, oth, own)
            kh8[g * HG + 4 + j, pl.ds(r0, KQR // 4), :] = jnp.where(hi_half, own, oth)

    def kquant_steps(i, invs, st, lo, hi, pace):
        for sidx in range(lo, hi):
            if sidx < nz:
                inv = invs[sidx // zpg]
                if pace is not None:
                    pr = (sidx - lo) * (pace.shape[0] // 8) // (hi - lo) * 8
                    inv = _tie(inv, pace[pr:pr + 8])
                st[sidx] = kq0(i, sidx // zpg, sidx % zpg, inv)
            if 0 <= sidx - 1 < nz:
                st[sidx - 1] = kq1(st[sidx - 1])
            if 0 <= sidx - 2 < nz:
                st[sidx - 2] = kq2(st[sidx - 2])
            if 0 <= sidx - 3 < nz:
                kq3(i, (sidx - 3) // zpg, (sidx - 3) % zpg, st.pop(sidx - 3))

    def qdot(i, n):
        xn = pltpu.bitcast(xn_s[i, n * 64:(n + 1) * 64, :], _BF)
        qt_ = _nt_dot(pltpu.bitcast(wqvt[0], _BF), xn)
        ls = slice(n * 128, (n + 1) * 128)
        for h in range(H):
            q = qt_[h * DH:(h + 1) * DH]
            qm = jnp.maximum(jnp.max(jnp.abs(q), axis=0, keepdims=True), 1e-30)
            sq[i, h:h + 1, ls] = qm * qscale
            u = q * (127.0 * _recip(qm))
            ai = _rnd(u)
            bi = _rnd((u - ai.astype(_F32)) * float(NREP * 2 ** SC))
            asi = _rnd(u * (2.0 ** -SA))
            xx = [asi, bi] if h % 2 == 0 else [bi, asi]
            qw[i, h, :, ls] = _pack8(jnp.concatenate([ai, ai] + xx, axis=0))

    def vdot(i, n):
        xn = pltpu.bitcast(xn_s[i, n * 64:(n + 1) * 64, :], _BF)
        v = _nt_dot(pltpu.bitcast(wqvt[1], _BF), xn)
        vt[i, :, n * 128:(n + 1) * 128] = v
        return v

    def pace_rows(a, k, nk):
        span = a.shape[0] // nk
        return jnp.concatenate(
            [a[k * span + r * span // 128 * 8:k * span + r * span // 128 * 8 + 8]
             for r in range(16)], axis=0)

    x_copy(0).wait()
    for n in range(nsub):
        ln1(0, n, None)
    wqkv_copy(1).wait()
    kdot(0, 0)
    kdot(0, 1)
    x_copy(1).wait()
    kg = kdot(0, 2)
    for n in range(nsub):
        ln1(1, n, pace_rows(kg, n, nsub))
    kdot(0, 3)
    for i in range(1, nt):
        if i + 1 < nt:
            x_copy(i + 1).wait()
        if i == nt - 2:
            wqkv_copy(2).wait()
        if i == nt - 1:
            wqkv_copy(0).wait()
        for g in range(ng):
            kg = kdot(i, g)
            if i + 1 < nt and g < 2:
                ln1(i + 1, 2 * g, pace_rows(kg, 0, 2))
                ln1(i + 1, 2 * g + 1, pace_rows(kg, 1, 2))
        if i == nt - 2:
            wqvt[1] = pltpu.bitcast(wqkv_v[2].T, _U32)
        if i == nt - 1:
            wqvt[0] = pltpu.bitcast(wqkv_v[0].T, _U32)

    def phase1b(ii, carry):
        for u in range(P1U):
            i = ii * P1U + u
            invs = [kscale(i, g) for g in range(ng)]
            st = {}
            for n in range(nsub):
                v = vdot(i, n)
                kquant_steps(i, invs, st, n * zpg, (n + 1) * zpg, v)
            kquant_steps(i, invs, st, nz, nz + 3, None)
            for n in range(nsub):
                qdot(i, n)
        return carry

    lax.fori_loop(0, nt // P1U, phase1b, 0)

    nf = S // KF
    fpt = TQ // KF
    bpt = ng // GP
    nbody = nt * bpt

    def scores(i, j, c):
        qi = i // bpt
        h = (i % bpt) * (GP * HG) + j
        w2 = qw[qi, h]
        aa, xx = w2[0:8], w2[8:16]
        w = jnp.concatenate([xx if r == (j % HG) // 2 else aa for r in range(4)], axis=0)
        kc = kh8[h, c * (KF // 4):(c + 1) * (KF // 4), :]
        return jnp.dot(pltpu.bitcast(kc, _I8), pltpu.bitcast(w, _I8),
                       preferred_element_type=_I32)

    if CARRY:
        scar[...] = scores(0, 0, 0)

    def fast_body(i, carry):
        lmax, lmin = carry
        qi = i // bpt
        n = GP * HG * nf
        pend = scar[...] if CARRY else scores(i, 0, 0)
        l8 = acc = sqb = cs = None
        for t in range(n):
            s = pend
            if t + 1 < n:
                pend = scores(i, (t + 1) // nf, (t + 1) % nf)
            elif CARRY:
                scar[...] = scores(jnp.minimum(i + 1, nbody - 1), 0, 0)
            j, c = t // nf, t % nf
            h = (i % bpt) * (GP * HG) + j
            if c == 0:
                l8 = acc = None
                sqb = jnp.broadcast_to(sq[qi, pl.ds(h, 1), :], (8, TQ))
            if c % fpt == 0:
                sk = skb[c // fpt, h]
                cs = sqb * jnp.concatenate([sk] * nsub, axis=1)
            p3 = jnp.exp2(s.astype(_F32).reshape(KF // 8, 8, TQ) * cs[None])
            for r in range(KF // 8):
                l8 = p3[r] if l8 is None else l8 + p3[r]
            p = jnp.concatenate([p3[b * 16 + r] for b in range(KF // 128)
                                 for r in range(15, -1, -1)], axis=0)
            v = vt[c // fpt, pl.ds(pl.multiple_of(h * DH, DH), DH), pl.ds((c % fpt) * KF, KF)]
            if BFP:
                v = v.astype(_BF); p = p.astype(_BF)
            pv = jnp.dot(v, p, preferred_element_type=_F32)
            acc = pv if acc is None else pv + acc
            if c == nf - 1:
                l = jnp.sum(l8, axis=0, keepdims=True)
                for z in range(nsub):
                    lz = l[:, z * 128:(z + 1) * 128]
                    lmax = jnp.maximum(lmax, lz)
                    lmin = jnp.minimum(lmin, lz)
                ot[qi, pl.ds(pl.multiple_of(h * (DH // 2), DH // 2), DH // 2), :] = (
                    pltpu.bitcast((acc * _recip(l)).astype(_BF), _U32))
        return lmax, lmin

    lmax, lmin = lax.fori_loop(
        0, nbody, fast_body, (jnp.ones((1, 128), _F32), jnp.ones((1, 128), _F32)))
    sqm = jnp.max(jnp.max(sq[...], axis=0), axis=1, keepdims=True)
    skm = jnp.max(skb[:, :, 0, :], axis=0)
    cmax = jnp.max(sqm * skm, axis=0, keepdims=True)
    okv = ((cmax <= CMAX / (NREP * 127.0 * 127.0)) & (lmax <= LMAX) & (lmin >= 1.0 / LMAX))
    n_ok = jnp.sum(jnp.where(okv, 1.0, 0.0))
    use_slow = n_ok < (129.0 if FORCE_SLOW else 128.0)

    @pl.when(use_slow)
    def _():
        nc = S // KC
        cpt = TQ // KC

        def prep(z, carry):
            i = z // nsub
            r2 = pl.multiple_of((z % nsub) * 64, 64)
            xn = pltpu.bitcast(xn_s[i, pl.ds(r2, 64), :], _BF)
            kf = jnp.dot(xn, wqkv_v[1], preferred_element_type=_F32)
            ku = pltpu.bitcast(kf.astype(_BF), _U32)
            rh = pl.multiple_of(z * 64, 64)
            for g in range(ng):
                kg = ku[:, g * 128:(g + 1) * 128]
                for j in range(HG):
                    kr = kg if j == 0 else pltpu.roll(kg, 128 - DH * j, axis=1)
                    kh[g * HG + j, pl.ds(rh, 64), :] = kr
            q = _nt_dot(pltpu.bitcast(wqvt[0], _BF), xn)
            qt[z] = pltpu.bitcast((q * qscale).astype(_BF), _U32)
            return carry

        lax.fori_loop(0, nt * nsub, prep, 0)

        def item(it, carry):
            h = it % H
            qi = it // H
            hr = pl.multiple_of(h * (DH // 2), DH // 2)
            q = pltpu.bitcast(jnp.concatenate(
                [qt[qi * nsub + n, pl.ds(hr, DH // 2), :] for n in range(nsub)], axis=1), _BF)

            def pass1(c, m8):
                kr = pl.multiple_of(c * (KC // 2), KC // 2)
                kc = pltpu.bitcast(kh[h, pl.ds(kr, KC // 2), :], _BF)[:, :DH]
                s = jnp.dot(kc, q, preferred_element_type=_F32)
                sbuf[c] = s
                return jnp.maximum(m8, jnp.max(s.reshape(KC // 8, 8, TQ), axis=0))

            m8 = lax.fori_loop(0, nc, pass1, jnp.full((8, TQ), -jnp.inf, _F32))
            m = jnp.max(m8, axis=0, keepdims=True)

            def pass2(ti, la):
                l8, acc = la
                for cc in range(cpt):
                    p = jnp.exp2(sbuf[ti * cpt + cc] - m)
                    l8 = l8 + jnp.sum(p.reshape(KC // 8, 8, TQ), axis=0)
                    v = vt[ti, pl.ds(pl.multiple_of(h * DH, DH), DH), cc * KC:(cc + 1) * KC]
                    acc = acc + jnp.dot(v, p, preferred_element_type=_F32)
                return l8, acc

            l8, acc = lax.fori_loop(0, nt, pass2,
                                    (jnp.zeros((8, TQ), _F32), jnp.zeros((DH, TQ), _F32)))
            o = acc * (1.0 / jnp.sum(l8, axis=0, keepdims=True))
            ot[qi, pl.ds(hr, DH // 2), :] = pltpu.bitcast(o.astype(_BF), _U32)
            return carry

        lax.fori_loop(0, nt * H, item, 0)

    for c in w_copies:
        c.wait()

    orows = TQ // OSPLIT

    def out_copy(i, k):
        r0 = pl.multiple_of(i * TQ + k * orows, orows)
        return pltpu.make_async_copy(obuf.at[pl.ds(r0, orows)], out_hbm.at[pl.ds(r0, orows)],
                                     sem_out.at[i * OSPLIT + k])

    def ln2(src, dst, pace):
        for n in range(nsub):
            dep = None if pace is None else pace_rows(pace, n, nsub)
            hn = _layernorm(hres_s[src, n * 128:(n + 1) * 128, :], dep).astype(_BF)
            xn_s[dst, n * 64:(n + 1) * 64, :] = pltpu.bitcast(hn, _U32)

    for i in range(nt):
        o_t = pltpu.bitcast(ot[i], _BF)
        attn = lax.dot_general(o_t, wo_v[...], (((0,), (0,)), ((), ())),
                               preferred_element_type=_F32)
        hres_s[i] = x_v[i * TQ:(i + 1) * TQ, :].astype(_F32) + attn
        if i == 1:
            ln2(0, 0, jnp.concatenate([attn[:, g * 128:(g + 1) * 128] for g in range(ng)], axis=0))

    def ffn(i, carry):
        hn = pltpu.bitcast(xn_s[i], _BF)
        acc = hres_s[i] + b2_ref[...].astype(_F32)[None, :]
        for f0 in range(0, F, FC):
            z = jnp.dot(hn, w1_v[:, f0:f0 + FC], preferred_element_type=_F32)
            z = _gelu(z + b1_ref[f0:f0 + FC].astype(_F32)[None, :]).astype(_BF)
            if f0 + FC < F:
                acc = jnp.dot(z, w2_v[f0:f0 + FC, :], preferred_element_type=_F32) + acc
                if f0 == 0:
                    ln2(jnp.minimum(i + 1, nt - 1), i + 1,
                        jnp.concatenate([acc[:, 0:128], acc[:, D - 128:D]], axis=0))
            else:
                for k in range(OSPLIT):
                    rs = slice(k * orows, (k + 1) * orows)
                    o = jnp.dot(z[rs], w2_v[f0:f0 + FC, :], preferred_element_type=_F32) + acc[rs]
                    r0 = pl.multiple_of(i * TQ + k * orows, orows)
                    obuf[pl.ds(r0, orows), :] = o.astype(obuf.dtype)
                    out_copy(i, k).start()
        return carry

    lax.fori_loop(0, nt, ffn, 0)
    for i in range(nt):
        for k in range(OSPLIT):
            out_copy(i, k).wait()


@jax.jit
def pallas_sequential_preLN__softmax_full_mha__dense_activation_gelu__prompt_kernel(
    A_x: jax.Array,
    A_wqkv: jax.Array,
    A_wo: jax.Array,
    B_x: jax.Array,
    B_w1: jax.Array,
    B_b1: jax.Array,
    B_w2: jax.Array,
    B_b2: jax.Array,
):
    B, S, D = A_x.shape
    F = B_w1.shape[1]
    assert B == 1 and D == H * DH
    nt = S // TQ
    x = A_x.reshape(S, D)
    any_spec = pl.BlockSpec(memory_space=pl.ANY)
    out = pl.pallas_call(
        functools.partial(_kernel, S=S, D=D, F=F),
        out_shape=jax.ShapeDtypeStruct((S, D), A_x.dtype),
        in_specs=[any_spec] * 7,
        out_specs=any_spec,
        scratch_shapes=[
            pltpu.VMEM((F,), _BF),
            pltpu.VMEM((D,), _BF),
            pltpu.VMEM((S, D), _BF),
            pltpu.VMEM((3, D, D), _BF),
            pltpu.VMEM((D, D), _BF),
            pltpu.VMEM((D, F), _BF),
            pltpu.VMEM((F, D), _BF),
            pltpu.VMEM((2, D // 2, D), _U32),
            pltpu.VMEM((nt + 1, TQ // 2, D), _U32),
            pltpu.VMEM((nt, D // 128, TQ, 128), _F32),
            pltpu.VMEM((nt, D // 128, 8, 128), _F32),
            pltpu.VMEM((H, S // 4, 128), _U32),
            pltpu.VMEM((nt, H, 16, TQ), _U32),
            pltpu.VMEM((nt, H, TQ), _F32),
            pltpu.VMEM((nt, H, 8, 128), _F32),
            pltpu.VMEM((nt, D, TQ), _F32),
            pltpu.VMEM((nt, D // 2, TQ), _U32),
            pltpu.VMEM((KF, TQ), _I32),
            pltpu.VMEM((nt, TQ, D), _F32),
            pltpu.VMEM((S, D), _BF),
            pltpu.VMEM((H, S // 2, 128), _U32),
            pltpu.VMEM((S // 128, D // 2, 128), _U32),
            pltpu.VMEM((S // KC, KC, TQ), _F32),
            pltpu.SemaphoreType.DMA((nt + 8,)),
            pltpu.SemaphoreType.DMA((nt * OSPLIT,)),
        ],
        compiler_params=pltpu.CompilerParams(vmem_limit_bytes=110 * 1024 * 1024),
    )(x, A_wqkv, A_wo, B_w1, B_w2, B_b1, B_b2)
    return out.reshape(B, S, D)
```

```python
import functools
import math

import jax
import jax.numpy as jnp
from jax import lax
import jax.experimental.pallas as pl
import jax.experimental.pallas.tpu as pltpu

_BF = jnp.bfloat16
_F32 = jnp.float32
_U32 = jnp.uint32
_I32 = jnp.int32
_I8 = jnp.int8

H = 32
DH = 16
HG = 128 // DH
TQ = 512
FC = 256
EPS = 1e-5

KF = 256
GP = 2
NREP = 6
SA = 3
SC = 2
CMAX = 32.0
LMAX = 2.0 ** 40
KQR = 64
P1U = 2
OSPLIT = 4

KC = 256


def _tie(val, dep):
    return jnp.where(pltpu.bitcast(dep, _I32) == 0x7FBADBAD, dep, val)


def _layernorm(x, dep=None):
    r, d = x.shape
    m = jnp.broadcast_to(jnp.mean(x, axis=-1, keepdims=True), (r, 128))
    if dep is not None:
        m = _tie(m, dep)
    xc = x - jnp.concatenate([m] * (d // 128), axis=1)
    v = jnp.mean(xc * xc, axis=-1, keepdims=True)
    return xc * lax.rsqrt(v + EPS)


def _gelu(x):
    c = math.sqrt(2.0 / math.pi)
    return 0.5 * x * (1.0 + jnp.tanh(c * (x + 0.044715 * (x * x * x))))


def _rnd(x):
    return jnp.round(x).astype(_I32)


def _recip(x):
    r = pl.reciprocal(x, approx=True)
    return r * (2.0 - x * r)


def _pack8(x):
    return pltpu.bitcast(x.astype(_I8), _U32)


def _nt_dot(a, b):
    return lax.dot_general(a, b, (((1,), (1,)), ((), ())), preferred_element_type=_F32)


def _pace_rows(a, k, nk):
    span = a.shape[0] // nk
    starts = [k * span + r * span // 128 * 8 for r in range(16)]
    return jnp.concatenate([a[s:s + 8] for s in starts], axis=0)


def _kernel(x_hbm, wqkv_hbm, wo_hbm, w1_hbm, w2_hbm, b1_hbm, b2_hbm, out_hbm,
            b1_v, b2_v, x_v, wqkv_v, wo_v, w1_v, w2_v, wqvt, xn_s, kf_s, cm_s,
            kh8, qw, sq, skb, vt, ot, hn_s, hres_s, obuf, kh, qt, sbuf,
            sem_in, sem_out, *, S, D, F):
    nt = S // TQ
    nsub = TQ // 128
    ng = D // 128
    assert nt == 4 and ng == 4 and nsub == 4
    qscale = (DH ** -0.5) * math.log2(math.e)

    def x_copy(i):
        return pltpu.make_async_copy(x_hbm.at[pl.ds(i * TQ, TQ)], x_v.at[pl.ds(i * TQ, TQ)],
                                     sem_in.at[i])

    def wqkv_copy(j):
        return pltpu.make_async_copy(wqkv_hbm.at[:, pl.ds(j * D, D)], wqkv_v.at[j],
                                     sem_in.at[nt + j])

    late_copies = [
        pltpu.make_async_copy(src, dst, sem_in.at[nt + 3])
        for src, dst in ((wo_hbm, wo_v), (w1_hbm, w1_v), (w2_hbm, w2_v),
                         (b1_hbm, b1_v), (b2_hbm, b2_v))]
    x_copy(0).start()
    wqkv_copy(1).start()
    for i in range(1, nt):
        x_copy(i).start()
    wqkv_copy(2).start()
    wqkv_copy(0).start()
    for c in late_copies:
        c.start()

    def ln1(i, n, dep):
        r0 = i * TQ + n * 128
        xn = _layernorm(x_v[r0:r0 + 128, :].astype(_F32), dep).astype(_BF)
        xn_s[i, n * 64:(n + 1) * 64, :] = pltpu.bitcast(xn, _U32)

    def kdot(i, g):
        kg = jnp.dot(pltpu.bitcast(xn_s[i], _BF), wqkv_v[1, :, g * 128:(g + 1) * 128],
                     preferred_element_type=_F32)
        kf_s[i, g] = kg
        cm_s[i, g] = jnp.max(jnp.abs(kg).reshape(TQ // 8, 8, 128), axis=0)
        return kg

    x_copy(0).wait()
    for n in range(nsub):
        ln1(0, n, None)
    wqkv_copy(1).wait()
    kdot(0, 0)
    kdot(0, 1)
    x_copy(1).wait()
    kg = kdot(0, 2)
    for n in range(nsub):
        ln1(1, n, _pace_rows(kg, n, nsub))
    kdot(0, 3)
    x_copy(2).wait()
    for g in range(ng):
        kg = kdot(1, g)
        if g < 2:
            ln1(2, 2 * g, _pace_rows(kg, 0, 2))
            ln1(2, 2 * g + 1, _pace_rows(kg, 1, 2))
    kdot(2, 0)
    x_copy(3).wait()
    wqkv_copy(2).wait()
    wqkv_copy(0).wait()
    for g in range(1, ng):
        kg = kdot(2, g)
        if g < 3:
            ln1(3, 2 * g - 2, _pace_rows(kg, 0, 2))
            ln1(3, 2 * g - 1, _pace_rows(kg, 1, 2))
    for g in range(ng):
        kdot(3, g)
    wqvt[1] = pltpu.bitcast(wqkv_v[2].T, _U32)
    wqvt[0] = pltpu.bitcast(wqkv_v[0].T, _U32)

    blk8 = lax.broadcasted_iota(_I32, (8, 128), 1) // DH
    blk = lax.broadcasted_iota(_I32, (KQR // 4, 128), 1) // DH
    odd_blk = (blk & 1) == 1
    odd_pair = (blk & 2) == 2
    hi_half = blk >= 4
    zpg = TQ // KQR
    nz = ng * zpg

    def kscale(i, g):
        cm = cm_s[i, g]
        mx = None
        for j in range(HG):
            mh = jnp.max(jnp.where(blk8 == j, cm, 0.0), axis=1, keepdims=True)
            mh = jnp.maximum(jnp.max(mh, axis=0, keepdims=True), 1e-30)
            mh = jnp.broadcast_to(mh, (8, 128))
            skb[i, g * HG + j] = mh * (1.0 / (NREP * 127.0 * 127.0))
            mx = mh if mx is None else jnp.where(blk8 == j, mh, mx)
        return 127.0 * _recip(mx)

    def kq0(i, g, z, inv):
        b0 = (z * KQR) // 128 * 128
        src = b0 + 128 - (z * KQR - b0) - KQR
        w = kf_s[i, g, src:src + KQR, :].reshape(KQR // 8, 8, 128) * inv[None]
        w = jnp.concatenate([w[r] for r in range(KQR // 8 - 1, -1, -1)], axis=0)
        ci = _rnd(w)
        c = _pack8(ci)
        d = _pack8(_rnd((w - ci.astype(_F32)) * float(NREP * 2 ** SA)))
        cs = _pack8(_rnd(w * (2.0 ** -SC)))
        return (c, d, pltpu.roll(c, 16, axis=1), pltpu.roll(c, 112, axis=1),
                pltpu.roll(cs, 16, axis=1), pltpu.roll(cs, 112, axis=1))

    def kq1(st):
        c, d, cu, cd, su, sd = st
        a_e = [jnp.where(odd_blk, cu, c), jnp.where(odd_blk, c, cd)]
        e_e = [jnp.where(odd_blk, su, d), jnp.where(odd_blk, d, sd)]
        return [(a_e[e], e_e[e], pltpu.roll(a_e[e], 32, axis=1), pltpu.roll(a_e[e], 96, axis=1))
                for e in range(2)]

    def kq2(st):
        out = []
        for e in range(2):
            a, ee, up, dn = st[e]
            out.append((e, jnp.where(odd_pair, up, ee),
                        pltpu.roll(jnp.where(odd_pair, up, a), 64, axis=1)))
            out.append((2 + e, jnp.where(odd_pair, ee, dn),
                        pltpu.roll(jnp.where(odd_pair, a, dn), 64, axis=1)))
        return out

    def kq3(i, g, z, st):
        r0 = pl.multiple_of(i * (TQ // 4) + z * (KQR // 4), KQR // 4)
        for j, own, oth in st:
            kh8[g * HG + j, pl.ds(r0, KQR // 4), :] = jnp.where(hi_half, oth, own)
            kh8[g * HG + 4 + j, pl.ds(r0, KQR // 4), :] = jnp.where(hi_half, own, oth)

    def ksplit_steps(i, invs, st, lo, hi, pace):
        for s in range(lo, hi):
            if s < nz:
                pr = (s - lo) * (pace.shape[0] // 8) // (hi - lo) * 8
                st[s] = kq0(i, s // zpg, s % zpg, _tie(invs[s // zpg], pace[pr:pr + 8]))
            if 0 <= s - 1 < nz:
                st[s - 1] = kq1(st[s - 1])
            if 0 <= s - 2 < nz:
                st[s - 2] = kq2(st[s - 2])
            if 0 <= s - 3 < nz:
                kq3(i, (s - 3) // zpg, (s - 3) % zpg, st.pop(s - 3))

    def vdot(i, n):
        xn = pltpu.bitcast(xn_s[i, n * 64:(n + 1) * 64, :], _BF)
        v = _nt_dot(pltpu.bitcast(wqvt[1], _BF), xn)
        vt[i, :, n * 128:(n + 1) * 128] = v
        return v

    def qdot(i, n):
        xn = pltpu.bitcast(xn_s[i, n * 64:(n + 1) * 64, :], _BF)
        qt_ = _nt_dot(pltpu.bitcast(wqvt[0], _BF), xn)
        ls = slice(n * 128, (n + 1) * 128)
        for h in range(H):
            q = qt_[h * DH:(h + 1) * DH]
            qm = jnp.maximum(jnp.max(jnp.abs(q), axis=0, keepdims=True), 1e-30)
            sq[i, h:h + 1, ls] = qm * qscale
            u = q * (127.0 * _recip(qm))
            ai = _rnd(u)
            bi = _rnd((u - ai.astype(_F32)) * float(NREP * 2 ** SC))
            asi = _rnd(u * (2.0 ** -SA))
            xx = [asi, bi] if h % 2 == 0 else [bi, asi]
            qw[i, h, :, ls] = _pack8(jnp.concatenate([ai, ai] + xx, axis=0))

    def phase1b(ii, carry):
        for u in range(P1U):
            i = ii * P1U + u
            invs = [kscale(i, g) for g in range(ng)]
            st = {}
            for n in range(nsub):
                ksplit_steps(i, invs, st, n * zpg, (n + 1) * zpg, vdot(i, n))
            ksplit_steps(i, invs, st, nz, nz + 3, None)
            for n in range(nsub):
                qdot(i, n)
        return carry

    lax.fori_loop(0, nt // P1U, phase1b, 0)
    for c in late_copies:
        c.wait()

    nf = S // KF
    fpt = TQ // KF
    bpt = ng // GP
    nstep = GP * HG * nf

    def fast_body(i, carry):
        lmax, lmin = carry
        qi = i // bpt
        h0 = (i % bpt) * (GP * HG)

        def scores(t):
            j, c = t // nf, t % nf
            w2 = qw[qi, h0 + j]
            aa, xx = w2[0:8], w2[8:16]
            w = jnp.concatenate([xx if r == (j % HG) // 2 else aa for r in range(4)], axis=0)
            kc = kh8[h0 + j, c * (KF // 4):(c + 1) * (KF // 4), :]
            return jnp.dot(pltpu.bitcast(kc, _I8), pltpu.bitcast(w, _I8),
                           preferred_element_type=_I32)

        pend = scores(0)
        l8 = acc = sqb = cs = None
        for t in range(nstep):
            s = pend
            if t + 1 < nstep:
                pend = scores(t + 1)
            c = t % nf
            h = h0 + t // nf
            if c == 0:
                l8 = acc = None
                sqb = jnp.broadcast_to(sq[qi, pl.ds(h, 1), :], (8, TQ))
            if c % fpt == 0:
                cs = sqb * jnp.concatenate([skb[c // fpt, h]] * nsub, axis=1)
            p3 = jnp.exp2(s.astype(_F32).reshape(KF // 8, 8, TQ) * cs[None])
            for r in range(KF // 8):
                l8 = p3[r] if l8 is None else l8 + p3[r]
            p = jnp.concatenate([p3[b * 16 + r] for b in range(KF // 128)
                                 for r in range(15, -1, -1)], axis=0)
            v = vt[c // fpt, pl.ds(pl.multiple_of(h * DH, DH), DH), pl.ds((c % fpt) * KF, KF)]
            pv = jnp.dot(v, p, preferred_element_type=_F32)
            acc = pv if acc is None else pv + acc
            if c == nf - 1:
                l = jnp.sum(l8, axis=0, keepdims=True)
                for z in range(nsub):
                    lz = l[:, z * 128:(z + 1) * 128]
                    lmax = jnp.maximum(lmax, lz)
                    lmin = jnp.minimum(lmin, lz)
                ot[qi, pl.ds(pl.multiple_of(h * (DH // 2), DH // 2), DH // 2), :] = (
                    pltpu.bitcast((acc * _recip(l)).astype(_BF), _U32))
        return lmax, lmin

    lmax, lmin = lax.fori_loop(
        0, nt * bpt, fast_body, (jnp.ones((1, 128), _F32), jnp.ones((1, 128), _F32)))

    def fast_path_unsafe():
        sqm = jnp.max(jnp.max(sq[...], axis=0), axis=1, keepdims=True)
        skm = jnp.max(skb[:, :, 0, :], axis=0)
        cmax = jnp.max(sqm * skm, axis=0, keepdims=True)
        ok = ((cmax <= CMAX / (NREP * 127.0 * 127.0)) & (lmax <= LMAX) & (lmin >= 1.0 / LMAX))
        return jnp.sum(jnp.where(ok, 1.0, 0.0)) < 128.0

    def slow_attention():
        cpt = TQ // KC

        def prep(z, carry):
            r2 = pl.multiple_of((z % nsub) * 64, 64)
            xn = pltpu.bitcast(xn_s[z // nsub, pl.ds(r2, 64), :], _BF)
            kf = jnp.dot(xn, wqkv_v[1], preferred_element_type=_F32)
            ku = pltpu.bitcast(kf.astype(_BF), _U32)
            rh = pl.multiple_of(z * 64, 64)
            for g in range(ng):
                kg = ku[:, g * 128:(g + 1) * 128]
                for j in range(HG):
                    kr = kg if j == 0 else pltpu.roll(kg, 128 - DH * j, axis=1)
                    kh[g * HG + j, pl.ds(rh, 64), :] = kr
            q = _nt_dot(pltpu.bitcast(wqvt[0], _BF), xn)
            qt[z] = pltpu.bitcast((q * qscale).astype(_BF), _U32)
            return carry

        lax.fori_loop(0, nt * nsub, prep, 0)

        def item(it, carry):
            h = it % H
            qi = it // H
            hr = pl.multiple_of(h * (DH // 2), DH // 2)
            q = pltpu.bitcast(jnp.concatenate(
                [qt[qi * nsub + n, pl.ds(hr, DH // 2), :] for n in range(nsub)], axis=1), _BF)

            def pass1(c, m8):
                kr = pl.multiple_of(c * (KC // 2), KC // 2)
                kc = pltpu.bitcast(kh[h, pl.ds(kr, KC // 2), :], _BF)[:, :DH]
                s = jnp.dot(kc, q, preferred_element_type=_F32)
                sbuf[c] = s
                return jnp.maximum(m8, jnp.max(s.reshape(KC // 8, 8, TQ), axis=0))

            m8 = lax.fori_loop(0, S // KC, pass1, jnp.full((8, TQ), -jnp.inf, _F32))
            m = jnp.max(m8, axis=0, keepdims=True)

            def pass2(ti, la):
                l8, acc = la
                for cc in range(cpt):
                    p = jnp.exp2(sbuf[ti * cpt + cc] - m)
                    l8 = l8 + jnp.sum(p.reshape(KC // 8, 8, TQ), axis=0)
                    v = vt[ti, pl.ds(pl.multiple_of(h * DH, DH), DH), cc * KC:(cc + 1) * KC]
                    acc = acc + jnp.dot(v, p, preferred_element_type=_F32)
                return l8, acc

            l8, acc = lax.fori_loop(0, nt, pass2,
                                    (jnp.zeros((8, TQ), _F32), jnp.zeros((DH, TQ), _F32)))
            o = acc * (1.0 / jnp.sum(l8, axis=0, keepdims=True))
            ot[qi, pl.ds(hr, DH // 2), :] = pltpu.bitcast(o.astype(_BF), _U32)
            return carry

        lax.fori_loop(0, nt * H, item, 0)

    def ln2(i, pace):
        for n in range(nsub):
            hn = _layernorm(hres_s[i, n * 128:(n + 1) * 128, :], _pace_rows(pace, n, nsub))
            hn_s[0, n * 64:(n + 1) * 64, :] = pltpu.bitcast(hn.astype(_BF), _U32)

    def wo_stage(c):
        pl.when(c[0] == 1)(slow_attention)
        for i in range(nt):
            attn = lax.dot_general(pltpu.bitcast(ot[i], _BF), wo_v[...],
                                   (((0,), (0,)), ((), ())), preferred_element_type=_F32)
            hres_s[i] = x_v[i * TQ:(i + 1) * TQ, :].astype(_F32) + attn
            if i == 1:
                ln2(0, jnp.concatenate([attn[:, g * 128:(g + 1) * 128] for g in range(ng)],
                                       axis=0))
        return c[0] + 1, jnp.where(fast_path_unsafe(), 2, 1).astype(_I32)

    lax.while_loop(lambda c: c[0] < c[1], wo_stage, (jnp.int32(0), jnp.int32(1)))

    orows = TQ // OSPLIT

    def out_copy(i, k):
        r0 = pl.multiple_of(i * TQ + k * orows, orows)
        return pltpu.make_async_copy(obuf.at[pl.ds(r0, orows)], out_hbm.at[pl.ds(r0, orows)],
                                     sem_out.at[0])

    def ffn(i, carry):
        hn_u = hn_s[0]
        hn_s[1] = hn_u
        acc = hres_s[i] + b2_v[...].astype(_F32)[None, :]
        for f0 in range(0, F, FC):
            hn = pltpu.bitcast(hn_u if f0 == 0 else hn_s[1], _BF)
            z = jnp.dot(hn, w1_v[:, f0:f0 + FC], preferred_element_type=_F32)
            z = _gelu(z + b1_v[f0:f0 + FC].astype(_F32)[None, :]).astype(_BF)
            if f0 + FC < F:
                acc = jnp.dot(z, w2_v[f0:f0 + FC, :], preferred_element_type=_F32) + acc
                if f0 == 0:
                    ln2(jnp.minimum(i + 1, nt - 1),
                        jnp.concatenate([acc[:, 0:128], acc[:, D - 128:D]], axis=0))
            else:
                for k in range(OSPLIT):
                    rs = slice(k * orows, (k + 1) * orows)
                    o = jnp.dot(z[rs], w2_v[f0:f0 + FC, :], preferred_element_type=_F32) + acc[rs]
                    r0 = pl.multiple_of(i * TQ + k * orows, orows)
                    obuf[pl.ds(r0, orows), :] = o.astype(obuf.dtype)
                    out_copy(i, k).start()
        return carry

    lax.fori_loop(0, nt, ffn, 0)
    for i in range(nt):
        for k in range(OSPLIT):
            out_copy(i, k).wait()


@jax.jit
def pallas_sequential_preLN__softmax_full_mha__dense_activation_gelu__prompt_kernel(
    A_x: jax.Array,
    A_wqkv: jax.Array,
    A_wo: jax.Array,
    B_x: jax.Array,
    B_w1: jax.Array,
    B_b1: jax.Array,
    B_w2: jax.Array,
    B_b2: jax.Array,
):
    del B_x
    B, S, D = A_x.shape
    F = B_w1.shape[1]
    assert B == 1 and D == H * DH
    nt = S // TQ
    any_spec = pl.BlockSpec(memory_space=pl.ANY)
    out = pl.pallas_call(
        functools.partial(_kernel, S=S, D=D, F=F),
        out_shape=jax.ShapeDtypeStruct((S, D), A_x.dtype),
        in_specs=[any_spec] * 7,
        out_specs=any_spec,
        scratch_shapes=[
            pltpu.VMEM((F,), _BF),
            pltpu.VMEM((D,), _BF),
            pltpu.VMEM((S, D), _BF),
            pltpu.VMEM((3, D, D), _BF),
            pltpu.VMEM((D, D), _BF),
            pltpu.VMEM((D, F), _BF),
            pltpu.VMEM((F, D), _BF),
            pltpu.VMEM((2, D // 2, D), _U32),
            pltpu.VMEM((nt, TQ // 2, D), _U32),
            pltpu.VMEM((nt, D // 128, TQ, 128), _F32),
            pltpu.VMEM((nt, D // 128, 8, 128), _F32),
            pltpu.VMEM((H, S // 4, 128), _U32),
            pltpu.VMEM((nt, H, 16, TQ), _U32),
            pltpu.VMEM((nt, H, TQ), _F32),
            pltpu.VMEM((nt, H, 8, 128), _F32),
            pltpu.VMEM((nt, D, TQ), _F32),
            pltpu.VMEM((nt, D // 2, TQ), _U32),
            pltpu.VMEM((2, TQ // 2, D), _U32),
            pltpu.VMEM((nt, TQ, D), _F32),
            pltpu.VMEM((S, D), _BF),
            pltpu.VMEM((H, S // 2, 128), _U32),
            pltpu.VMEM((S // 128, D // 2, 128), _U32),
            pltpu.VMEM((S // KC, KC, TQ), _F32),
            pltpu.SemaphoreType.DMA((nt + 4,)),
            pltpu.SemaphoreType.DMA((1,)),
        ],
        compiler_params=pltpu.CompilerParams(vmem_limit_bytes=110 * 1024 * 1024),
    )(A_x.reshape(S, D), A_wqkv, A_wo, B_w1, B_w2, B_b1, B_b2)
    return out.reshape(B, S, D)
```

```python
import functools
import math

import jax
import jax.numpy as jnp
from jax import lax
import jax.experimental.pallas as pl
import jax.experimental.pallas.tpu as pltpu

_BF = jnp.bfloat16
_F32 = jnp.float32
_U32 = jnp.uint32
_I32 = jnp.int32
_I8 = jnp.int8

H = 32
DH = 16
HG = 128 // DH
TQ = 512
FC = 256
EPS = 1e-5

KF = 256
GP = 2
NREP = 6
SA = 3
SC = 2
CMAX = 32.0
LMAX = 2.0 ** 40
KQR = 64
P1U = 2
OSPLIT = 8

KC = 256


def _tie(val, dep):
    return jnp.where(pltpu.bitcast(dep, _I32) == 0x7FBADBAD, dep, val)


def _layernorm(x, dep=None):
    r, d = x.shape
    m = jnp.broadcast_to(jnp.mean(x, axis=-1, keepdims=True), (r, 128))
    if dep is not None:
        m = _tie(m, dep)
    xc = x - jnp.concatenate([m] * (d // 128), axis=1)
    v = jnp.mean(xc * xc, axis=-1, keepdims=True)
    return xc * lax.rsqrt(v + EPS)


def _gelu(x):
    c = math.sqrt(2.0 / math.pi)
    return 0.5 * x * (1.0 + jnp.tanh(c * (x + 0.044715 * (x * x * x))))


def _rnd(x):
    return jnp.round(x).astype(_I32)


def _recip(x):
    r = pl.reciprocal(x, approx=True)
    return r * (2.0 - x * r)


def _pack8(x):
    return pltpu.bitcast(x.astype(_I8), _U32)


def _nt_dot(a, b):
    return lax.dot_general(a, b, (((1,), (1,)), ((), ())), preferred_element_type=_F32)


def _pace_rows(a, k, nk):
    span = a.shape[0] // nk
    starts = [k * span + r * span // 128 * 8 for r in range(16)]
    return jnp.concatenate([a[s:s + 8] for s in starts], axis=0)


def _kernel(x_hbm, wqkv_hbm, wo_hbm, w1_hbm, w2_hbm, b1_hbm, b2_hbm, out_hbm,
            b1_v, b2_v, x_v, wqkv_v, wo_v, w1_v, w2_v, wqvt, xn_s, kf_s, cm_s,
            kh8, qw, sq, skb, vt, ot, hn_s, hres_s, obuf, kh, qt, sbuf,
            sem_in, sem_out, *, S, D, F):
    nt = S // TQ
    nsub = TQ // 128
    ng = D // 128
    assert nt == 4 and ng == 4 and nsub == 4
    qscale = (DH ** -0.5) * math.log2(math.e)

    def x_copy(i):
        return pltpu.make_async_copy(x_hbm.at[pl.ds(i * TQ, TQ)], x_v.at[pl.ds(i * TQ, TQ)],
                                     sem_in.at[i])

    def wqkv_copy(j):
        return pltpu.make_async_copy(wqkv_hbm.at[:, pl.ds(j * D, D)], wqkv_v.at[j],
                                     sem_in.at[nt + j])

    late_copies = [
        pltpu.make_async_copy(src, dst, sem_in.at[nt + 3])
        for src, dst in ((wo_hbm, wo_v), (w1_hbm, w1_v), (w2_hbm, w2_v),
                         (b1_hbm, b1_v), (b2_hbm, b2_v))]
    x_copy(0).start()
    wqkv_copy(1).start()
    for i in range(1, nt):
        x_copy(i).start()
    wqkv_copy(2).start()
    wqkv_copy(0).start()
    for c in late_copies:
        c.start()

    def ln1(i, n, dep):
        r0 = i * TQ + n * 128
        xn = _layernorm(x_v[r0:r0 + 128, :].astype(_F32), dep).astype(_BF)
        xn_s[i, n * 64:(n + 1) * 64, :] = pltpu.bitcast(xn, _U32)

    def kdot(i, g):
        kg = jnp.dot(pltpu.bitcast(xn_s[i], _BF), wqkv_v[1, :, g * 128:(g + 1) * 128],
                     preferred_element_type=_F32)
        kf_s[i, g] = kg
        cm_s[i, g] = jnp.max(jnp.abs(kg).reshape(TQ // 8, 8, 128), axis=0)
        return kg

    x_copy(0).wait()
    for n in range(nsub):
        ln1(0, n, None)
    wqkv_copy(1).wait()
    kdot(0, 0)
    kdot(0, 1)
    x_copy(1).wait()
    kg = jnp.concatenate([kdot(0, 2), kdot(0, 3)[:TQ // 2]], axis=0)
    for n in range(nsub):
        ln1(1, n, _pace_rows(kg, n, nsub))
    x_copy(2).wait()
    for g in range(ng):
        kg = kdot(1, g)
        if g < 2:
            ln1(2, 2 * g, _pace_rows(kg, 0, 2))
            ln1(2, 2 * g + 1, _pace_rows(kg, 1, 2))
    kdot(2, 0)
    kdot(2, 1)
    x_copy(3).wait()
    wqkv_copy(2).wait()
    wqkv_copy(0).wait()
    kg = jnp.concatenate([kdot(2, 2), kdot(2, 3)], axis=0)
    for n in range(nsub):
        ln1(3, n, _pace_rows(kg, n, nsub))
    for g in range(ng):
        kdot(3, g)
    wqvt[1] = pltpu.bitcast(wqkv_v[2].T, _U32)
    wqvt[0] = pltpu.bitcast(wqkv_v[0].T, _U32)

    blk8 = lax.broadcasted_iota(_I32, (8, 128), 1) // DH
    blk = lax.broadcasted_iota(_I32, (KQR // 4, 128), 1) // DH
    odd_blk = (blk & 1) == 1
    odd_pair = (blk & 2) == 2
    hi_half = blk >= 4
    zpg = TQ // KQR
    nz = ng * zpg

    def kscale(i, g):
        cm = cm_s[i, g]
        mx = None
        for j in range(HG):
            mh = jnp.max(jnp.where(blk8 == j, cm, 0.0), axis=1, keepdims=True)
            mh = jnp.maximum(jnp.max(mh, axis=0, keepdims=True), 1e-30)
            mh = jnp.broadcast_to(mh, (8, 128))
            skb[i, g * HG + j] = mh * (1.0 / (NREP * 127.0 * 127.0))
            mx = mh if mx is None else jnp.where(blk8 == j, mh, mx)
        return 127.0 * _recip(mx)

    def kq0(i, g, z, inv):
        b0 = (z * KQR) // 128 * 128
        src = b0 + 128 - (z * KQR - b0) - KQR
        w = kf_s[i, g, src:src + KQR, :].reshape(KQR // 8, 8, 128) * inv[None]
        w = jnp.concatenate([w[r] for r in range(KQR // 8 - 1, -1, -1)], axis=0)
        ci = _rnd(w)
        c = _pack8(ci)
        d = _pack8(_rnd((w - ci.astype(_F32)) * float(NREP * 2 ** SA)))
        cs = _pack8(_rnd(w * (2.0 ** -SC)))
        return (c, d, pltpu.roll(c, 16, axis=1), pltpu.roll(c, 112, axis=1),
                pltpu.roll(cs, 16, axis=1), pltpu.roll(cs, 112, axis=1))

    def kq1(st):
        c, d, cu, cd, su, sd = st
        a_e = [jnp.where(odd_blk, cu, c), jnp.where(odd_blk, c, cd)]
        e_e = [jnp.where(odd_blk, su, d), jnp.where(odd_blk, d, sd)]
        return [(a_e[e], e_e[e], pltpu.roll(a_e[e], 32, axis=1), pltpu.roll(a_e[e], 96, axis=1))
                for e in range(2)]

    def kq2(st):
        out = []
        for e in range(2):
            a, ee, up, dn = st[e]
            out.append((e, jnp.where(odd_pair, up, ee),
                        pltpu.roll(jnp.where(odd_pair, up, a), 64, axis=1)))
            out.append((2 + e, jnp.where(odd_pair, ee, dn),
                        pltpu.roll(jnp.where(odd_pair, a, dn), 64, axis=1)))
        return out

    def kq3(i, g, z, st):
        r0 = pl.multiple_of(i * (TQ // 4) + z * (KQR // 4), KQR // 4)
        for j, own, oth in st:
            kh8[g * HG + j, pl.ds(r0, KQR // 4), :] = jnp.where(hi_half, oth, own)
            kh8[g * HG + 4 + j, pl.ds(r0, KQR // 4), :] = jnp.where(hi_half, own, oth)

    def ksplit_steps(i, invs, st, lo, hi, pace):
        for s in range(lo, hi):
            if s < nz:
                pr = (s - lo) * (pace.shape[0] // 8) // (hi - lo) * 8
                st[s] = kq0(i, s // zpg, s % zpg, _tie(invs[s // zpg], pace[pr:pr + 8]))
            if 0 <= s - 1 < nz:
                st[s - 1] = kq1(st[s - 1])
            if 0 <= s - 2 < nz:
                st[s - 2] = kq2(st[s - 2])
            if 0 <= s - 3 < nz:
                kq3(i, (s - 3) // zpg, (s - 3) % zpg, st.pop(s - 3))

    def vdot(i, n):
        xn = pltpu.bitcast(xn_s[i, n * 64:(n + 1) * 64, :], _BF)
        v = _nt_dot(pltpu.bitcast(wqvt[1], _BF), xn)
        vt[i, :, n * 128:(n + 1) * 128] = v
        return v

    def qdot(i, n):
        xn = pltpu.bitcast(xn_s[i, n * 64:(n + 1) * 64, :], _BF)
        qt_ = _nt_dot(pltpu.bitcast(wqvt[0], _BF), xn)
        ls = slice(n * 128, (n + 1) * 128)
        for h in range(H):
            q = qt_[h * DH:(h + 1) * DH]
            qm = jnp.maximum(jnp.max(jnp.abs(q), axis=0, keepdims=True), 1e-30)
            sq[i, h:h + 1, ls] = qm * qscale
            u = q * (127.0 * _recip(qm))
            ai = _rnd(u)
            bi = _rnd((u - ai.astype(_F32)) * float(NREP * 2 ** SC))
            asi = _rnd(u * (2.0 ** -SA))
            xx = [asi, bi] if h % 2 == 0 else [bi, asi]
            qw[i, h, :, ls] = _pack8(jnp.concatenate([ai, ai] + xx, axis=0))

    def phase1b(ii, carry):
        for u in range(P1U):
            i = ii * P1U + u
            invs = [kscale(i, g) for g in range(ng)]
            st = {}
            for n in range(nsub):
                ksplit_steps(i, invs, st, n * zpg, (n + 1) * zpg, vdot(i, n))
            ksplit_steps(i, invs, st, nz, nz + 3, None)
            for n in range(nsub):
                qdot(i, n)
        return carry

    lax.fori_loop(0, nt // P1U, phase1b, 0)
    for c in late_copies:
        c.wait()

    nf = S // KF
    fpt = TQ // KF
    bpt = ng // GP
    nstep = GP * HG * nf

    def fast_body(i, carry):
        lmax, lmin = carry
        qi = i // bpt
        h0 = (i % bpt) * (GP * HG)

        def scores(t):
            j, c = t // nf, t % nf
            w2 = qw[qi, h0 + j]
            aa, xx = w2[0:8], w2[8:16]
            w = jnp.concatenate([xx if r == (j % HG) // 2 else aa for r in range(4)], axis=0)
            kc = kh8[h0 + j, c * (KF // 4):(c + 1) * (KF // 4), :]
            return jnp.dot(pltpu.bitcast(kc, _I8), pltpu.bitcast(w, _I8),
                           preferred_element_type=_I32)

        pend = scores(0)
        l8 = acc = sqb = cs = None
        for t in range(nstep):
            s = pend
            if t + 1 < nstep:
                pend = scores(t + 1)
            c = t % nf
            h = h0 + t // nf
            if c == 0:
                l8 = acc = None
                sqb = jnp.broadcast_to(sq[qi, pl.ds(h, 1), :], (8, TQ))
            if c % fpt == 0:
                cs = sqb * jnp.concatenate([skb[c // fpt, h]] * nsub, axis=1)
            p3 = jnp.exp2(s.astype(_F32).reshape(KF // 8, 8, TQ) * cs[None])
            for r in range(KF // 8):
                l8 = p3[r] if l8 is None else l8 + p3[r]
            p = jnp.concatenate([p3[b * 16 + r] for b in range(KF // 128)
                                 for r in range(15, -1, -1)], axis=0)
            v = vt[c // fpt, pl.ds(pl.multiple_of(h * DH, DH), DH), pl.ds((c % fpt) * KF, KF)]
            pv = jnp.dot(v, p, preferred_element_type=_F32)
            acc = pv if acc is None else pv + acc
            if c == nf - 1:
                l = jnp.sum(l8, axis=0, keepdims=True)
                for z in range(nsub):
                    lz = l[:, z * 128:(z + 1) * 128]
                    lmax = jnp.maximum(lmax, lz)
                    lmin = jnp.minimum(lmin, lz)
                ot[qi, pl.ds(pl.multiple_of(h * (DH // 2), DH // 2), DH // 2), :] = (
                    pltpu.bitcast((acc * _recip(l)).astype(_BF), _U32))
        return lmax, lmin

    lmax, lmin = lax.fori_loop(
        0, nt * bpt, fast_body, (jnp.ones((1, 128), _F32), jnp.ones((1, 128), _F32)))

    def fast_path_unsafe():
        sqm = jnp.max(jnp.max(sq[...], axis=0), axis=1, keepdims=True)
        skm = jnp.max(skb[:, :, 0, :], axis=0)
        cmax = jnp.max(sqm * skm, axis=0, keepdims=True)
        ok = ((cmax <= CMAX / (NREP * 127.0 * 127.0)) & (lmax <= LMAX) & (lmin >= 1.0 / LMAX))
        return jnp.sum(jnp.where(ok, 1.0, 0.0)) < 128.0

    def slow_attention():
        cpt = TQ // KC

        def prep(z, carry):
            r2 = pl.multiple_of((z % nsub) * 64, 64)
            xn = pltpu.bitcast(xn_s[z // nsub, pl.ds(r2, 64), :], _BF)
            kf = jnp.dot(xn, wqkv_v[1], preferred_element_type=_F32)
            ku = pltpu.bitcast(kf.astype(_BF), _U32)
            rh = pl.multiple_of(z * 64, 64)
            for g in range(ng):
                kg = ku[:, g * 128:(g + 1) * 128]
                for j in range(HG):
                    kr = kg if j == 0 else pltpu.roll(kg, 128 - DH * j, axis=1)
                    kh[g * HG + j, pl.ds(rh, 64), :] = kr
            q = _nt_dot(pltpu.bitcast(wqvt[0], _BF), xn)
            qt[z] = pltpu.bitcast((q * qscale).astype(_BF), _U32)
            return carry

        lax.fori_loop(0, nt * nsub, prep, 0)

        def item(it, carry):
            h = it % H
            qi = it // H
            hr = pl.multiple_of(h * (DH // 2), DH // 2)
            q = pltpu.bitcast(jnp.concatenate(
                [qt[qi * nsub + n, pl.ds(hr, DH // 2), :] for n in range(nsub)], axis=1), _BF)

            def pass1(c, m8):
                kr = pl.multiple_of(c * (KC // 2), KC // 2)
                kc = pltpu.bitcast(kh[h, pl.ds(kr, KC // 2), :], _BF)[:, :DH]
                s = jnp.dot(kc, q, preferred_element_type=_F32)
                sbuf[c] = s
                return jnp.maximum(m8, jnp.max(s.reshape(KC // 8, 8, TQ), axis=0))

            m8 = lax.fori_loop(0, S // KC, pass1, jnp.full((8, TQ), -jnp.inf, _F32))
            m = jnp.max(m8, axis=0, keepdims=True)

            def pass2(ti, la):
                l8, acc = la
                for cc in range(cpt):
                    p = jnp.exp2(sbuf[ti * cpt + cc] - m)
                    l8 = l8 + jnp.sum(p.reshape(KC // 8, 8, TQ), axis=0)
                    v = vt[ti, pl.ds(pl.multiple_of(h * DH, DH), DH), cc * KC:(cc + 1) * KC]
                    acc = acc + jnp.dot(v, p, preferred_element_type=_F32)
                return l8, acc

            l8, acc = lax.fori_loop(0, nt, pass2,
                                    (jnp.zeros((8, TQ), _F32), jnp.zeros((DH, TQ), _F32)))
            o = acc * (1.0 / jnp.sum(l8, axis=0, keepdims=True))
            ot[qi, pl.ds(hr, DH // 2), :] = pltpu.bitcast(o.astype(_BF), _U32)
            return carry

        lax.fori_loop(0, nt * H, item, 0)

    def ln2(i, pace):
        for n in range(nsub):
            hn = _layernorm(hres_s[i, n * 128:(n + 1) * 128, :], _pace_rows(pace, n, nsub))
            hn_s[0, n * 64:(n + 1) * 64, :] = pltpu.bitcast(hn.astype(_BF), _U32)

    def wo_stage(c):
        pl.when(c[0] == 1)(slow_attention)
        for i in range(nt):
            attn = lax.dot_general(pltpu.bitcast(ot[i], _BF), wo_v[...],
                                   (((0,), (0,)), ((), ())), preferred_element_type=_F32)
            hres_s[i] = x_v[i * TQ:(i + 1) * TQ, :].astype(_F32) + attn
            if i == 1:
                ln2(0, jnp.concatenate([attn[:, g * 128:(g + 1) * 128] for g in range(ng)],
                                       axis=0))
        return c[0] + 1, jnp.where(fast_path_unsafe(), 2, 1).astype(_I32)

    lax.while_loop(lambda c: c[0] < c[1], wo_stage, (jnp.int32(0), jnp.int32(1)))

    orows = TQ // OSPLIT

    def out_copy(i, k):
        r0 = pl.multiple_of(i * TQ + k * orows, orows)
        return pltpu.make_async_copy(obuf.at[pl.ds(r0, orows)], out_hbm.at[pl.ds(r0, orows)],
                                     sem_out.at[0])

    def ffn(i, carry):
        hn_u = hn_s[0]
        hn_s[1] = hn_u
        acc = hres_s[i] + b2_v[...].astype(_F32)[None, :]
        for f0 in range(0, F, FC):
            hn = pltpu.bitcast(hn_u if f0 == 0 else hn_s[1], _BF)
            z = jnp.dot(hn, w1_v[:, f0:f0 + FC], preferred_element_type=_F32)
            z = _gelu(z + b1_v[f0:f0 + FC].astype(_F32)[None, :]).astype(_BF)
            if f0 + FC < F:
                acc = jnp.dot(z, w2_v[f0:f0 + FC, :], preferred_element_type=_F32) + acc
                if f0 == 0:
                    ln2(jnp.minimum(i + 1, nt - 1),
                        jnp.concatenate([acc[:, 0:128], acc[:, D - 128:D]], axis=0))
            else:
                for k in range(OSPLIT):
                    rs = slice(k * orows, (k + 1) * orows)
                    o = jnp.dot(z[rs], w2_v[f0:f0 + FC, :], preferred_element_type=_F32) + acc[rs]
                    r0 = pl.multiple_of(i * TQ + k * orows, orows)
                    obuf[pl.ds(r0, orows), :] = o.astype(obuf.dtype)
                    out_copy(i, k).start()
        return carry

    lax.fori_loop(0, nt, ffn, 0)
    for i in range(nt):
        for k in range(OSPLIT):
            out_copy(i, k).wait()


@jax.jit
def pallas_sequential_preLN__softmax_full_mha__dense_activation_gelu__prompt_kernel(
    A_x: jax.Array,
    A_wqkv: jax.Array,
    A_wo: jax.Array,
    B_x: jax.Array,
    B_w1: jax.Array,
    B_b1: jax.Array,
    B_w2: jax.Array,
    B_b2: jax.Array,
):
    del B_x
    B, S, D = A_x.shape
    F = B_w1.shape[1]
    assert B == 1 and D == H * DH
    nt = S // TQ
    any_spec = pl.BlockSpec(memory_space=pl.ANY)
    out = pl.pallas_call(
        functools.partial(_kernel, S=S, D=D, F=F),
        out_shape=jax.ShapeDtypeStruct((S, D), A_x.dtype),
        in_specs=[any_spec] * 7,
        out_specs=any_spec,
        scratch_shapes=[
            pltpu.VMEM((F,), _BF),
            pltpu.VMEM((D,), _BF),
            pltpu.VMEM((S, D), _BF),
            pltpu.VMEM((3, D, D), _BF),
            pltpu.VMEM((D, D), _BF),
            pltpu.VMEM((D, F), _BF),
            pltpu.VMEM((F, D), _BF),
            pltpu.VMEM((2, D // 2, D), _U32),
            pltpu.VMEM((nt, TQ // 2, D), _U32),
            pltpu.VMEM((nt, D // 128, TQ, 128), _F32),
            pltpu.VMEM((nt, D // 128, 8, 128), _F32),
            pltpu.VMEM((H, S // 4, 128), _U32),
            pltpu.VMEM((nt, H, 16, TQ), _U32),
            pltpu.VMEM((nt, H, TQ), _F32),
            pltpu.VMEM((nt, H, 8, 128), _F32),
            pltpu.VMEM((nt, D, TQ), _F32),
            pltpu.VMEM((nt, D // 2, TQ), _U32),
            pltpu.VMEM((2, TQ // 2, D), _U32),
            pltpu.VMEM((nt, TQ, D), _F32),
            pltpu.VMEM((S, D), _BF),
            pltpu.VMEM((H, S // 2, 128), _U32),
            pltpu.VMEM((S // 128, D // 2, 128), _U32),
            pltpu.VMEM((S // KC, KC, TQ), _F32),
            pltpu.SemaphoreType.DMA((nt + 4,)),
            pltpu.SemaphoreType.DMA((1,)),
        ],
        compiler_params=pltpu.CompilerParams(vmem_limit_bytes=110 * 1024 * 1024),
    )(A_x.reshape(S, D), A_wqkv, A_wo, B_w1, B_w2, B_b1, B_b2)
    return out.reshape(B, S, D)
```

```python
import functools
import math

import jax
import jax.numpy as jnp
from jax import lax
import jax.experimental.pallas as pl
import jax.experimental.pallas.tpu as pltpu

_BF = jnp.bfloat16
_F32 = jnp.float32
_U32 = jnp.uint32
_I32 = jnp.int32
_I8 = jnp.int8

H = 32
DH = 16
HG = 128 // DH
TQ = 512
FC = 256
EPS = 1e-5

KF = 256
GP = 2
NREP = 6
SA = 3
SC = 2
CMAX = 32.0
LMAX = 2.0 ** 40
KQR = 64
P1U = 2
OSPLIT = 8

KC = 256


def _tie(val, dep):
    return jnp.where(pltpu.bitcast(dep, _I32) == 0x7FBADBAD, dep, val)


def _layernorm(x, dep=None):
    r, d = x.shape
    m = jnp.broadcast_to(jnp.mean(x, axis=-1, keepdims=True), (r, 128))
    if dep is not None:
        m = _tie(m, dep)
    xc = x - jnp.concatenate([m] * (d // 128), axis=1)
    v = jnp.mean(xc * xc, axis=-1, keepdims=True)
    return xc * lax.rsqrt(v + EPS)


def _gelu(x):
    c = math.sqrt(2.0 / math.pi)
    return 0.5 * x * (1.0 + jnp.tanh(c * (x + 0.044715 * (x * x * x))))


def _rnd(x):
    return jnp.round(x).astype(_I32)


def _recip(x):
    r = pl.reciprocal(x, approx=True)
    return r * (2.0 - x * r)


def _pack8(x):
    return pltpu.bitcast(x.astype(_I8), _U32)


def _nt_dot(a, b):
    return lax.dot_general(a, b, (((1,), (1,)), ((), ())), preferred_element_type=_F32)


def _tn_dot(a, b):
    return lax.dot_general(a, b, (((0,), (0,)), ((), ())), preferred_element_type=_F32)


def _pace_rows(a, k, nk):
    span = a.shape[0] // nk
    starts = [k * span + r * span // 128 * 8 for r in range(16)]
    return jnp.concatenate([a[s:s + 8] for s in starts], axis=0)


def _kernel(x_hbm, wqkv_hbm, wo_hbm, w1_hbm, w2_hbm, b1_hbm, b2_hbm, out_hbm,
            b1_v, b2_v, x_v, wqkv_v, wo_v, w1_v, w2_v, wqvt, xn_s, kf_s, cm_s,
            kh8, qw, sq, skb, vt, ot, hn_s, hres_s, obuf, kh, qt, sbuf,
            sem_in, sem_out, *, S, D, F):
    nt = S // TQ
    nsub = TQ // 128
    ng = D // 128
    assert nt == 4 and ng == 4 and nsub == 4 and GP == 2
    qscale = (DH ** -0.5) * math.log2(math.e)

    def x_copy(i):
        return pltpu.make_async_copy(x_hbm.at[pl.ds(i * TQ, TQ)], x_v.at[pl.ds(i * TQ, TQ)],
                                     sem_in.at[i])

    def wqkv_copy(j):
        return pltpu.make_async_copy(wqkv_hbm.at[:, pl.ds(j * D, D)], wqkv_v.at[j],
                                     sem_in.at[nt + j])

    late_copies = [
        pltpu.make_async_copy(src, dst, sem_in.at[nt + 3])
        for src, dst in ((wo_hbm, wo_v), (w1_hbm, w1_v), (w2_hbm, w2_v),
                         (b1_hbm, b1_v), (b2_hbm, b2_v))]
    x_copy(0).start()
    wqkv_copy(1).start()
    for i in range(1, nt):
        x_copy(i).start()
    wqkv_copy(2).start()
    wqkv_copy(0).start()
    for c in late_copies:
        c.start()

    def ln1(i, n, dep):
        r0 = i * TQ + n * 128
        x = x_v[r0:r0 + 128, :].astype(_F32)
        hres_s[i, n * 128:(n + 1) * 128, :] = x
        xn_s[i, n * 64:(n + 1) * 64, :] = pltpu.bitcast(_layernorm(x, dep).astype(_BF), _U32)

    def kdot(i, g):
        kg = jnp.dot(pltpu.bitcast(xn_s[i], _BF), wqkv_v[1, :, g * 128:(g + 1) * 128],
                     preferred_element_type=_F32)
        kf_s[i, g] = kg
        cm_s[i, g] = jnp.max(jnp.abs(kg).reshape(TQ // 8, 8, 128), axis=0)
        return kg

    x_copy(0).wait()
    for n in range(nsub):
        ln1(0, n, None)
    wqkv_copy(1).wait()
    kdot(0, 0)
    kdot(0, 1)
    x_copy(1).wait()
    kg = jnp.concatenate([kdot(0, 2), kdot(0, 3)[:TQ // 2]], axis=0)
    for n in range(nsub):
        ln1(1, n, _pace_rows(kg, n, nsub))
    x_copy(2).wait()
    for g in range(ng):
        kg = kdot(1, g)
        if g < 2:
            ln1(2, 2 * g, _pace_rows(kg, 0, 2))
            ln1(2, 2 * g + 1, _pace_rows(kg, 1, 2))
    kdot(2, 0)
    kdot(2, 1)
    x_copy(3).wait()
    wqkv_copy(2).wait()
    wqkv_copy(0).wait()
    kg = jnp.concatenate([kdot(2, 2), kdot(2, 3)], axis=0)
    for n in range(nsub):
        ln1(3, n, _pace_rows(kg, n, nsub))
    for g in range(ng):
        kdot(3, g)
    wqvt[1] = pltpu.bitcast(wqkv_v[2].T, _U32)
    wqvt[0] = pltpu.bitcast(wqkv_v[0].T, _U32)

    blk8 = lax.broadcasted_iota(_I32, (8, 128), 1) // DH
    blk = lax.broadcasted_iota(_I32, (KQR // 4, 128), 1) // DH
    odd_blk = (blk & 1) == 1
    odd_pair = (blk & 2) == 2
    hi_half = blk >= 4
    zpg = TQ // KQR
    nz = ng * zpg

    def kscale(i, g):
        cm = cm_s[i, g]
        mx = None
        for j in range(HG):
            mh = jnp.max(jnp.where(blk8 == j, cm, 0.0), axis=1, keepdims=True)
            mh = jnp.maximum(jnp.max(mh, axis=0, keepdims=True), 1e-30)
            mh = jnp.broadcast_to(mh, (8, 128))
            skb[i, g * HG + j] = mh * (1.0 / (NREP * 127.0 * 127.0))
            mx = mh if mx is None else jnp.where(blk8 == j, mh, mx)
        return 127.0 * _recip(mx)

    def kq0(i, g, z, inv):
        b0 = (z * KQR) // 128 * 128
        src = b0 + 128 - (z * KQR - b0) - KQR
        w = kf_s[i, g, src:src + KQR, :].reshape(KQR // 8, 8, 128) * inv[None]
        w = jnp.concatenate([w[r] for r in range(KQR // 8 - 1, -1, -1)], axis=0)
        ci = _rnd(w)
        c = _pack8(ci)
        d = _pack8(_rnd((w - ci.astype(_F32)) * float(NREP * 2 ** SA)))
        cs = _pack8(_rnd(w * (2.0 ** -SC)))
        return (c, d, pltpu.roll(c, 16, axis=1), pltpu.roll(c, 112, axis=1),
                pltpu.roll(cs, 16, axis=1), pltpu.roll(cs, 112, axis=1))

    def kq1(st):
        c, d, cu, cd, su, sd = st
        a_e = [jnp.where(odd_blk, cu, c), jnp.where(odd_blk, c, cd)]
        e_e = [jnp.where(odd_blk, su, d), jnp.where(odd_blk, d, sd)]
        return [(a_e[e], e_e[e], pltpu.roll(a_e[e], 32, axis=1), pltpu.roll(a_e[e], 96, axis=1))
                for e in range(2)]

    def kq2(st):
        out = []
        for e in range(2):
            a, ee, up, dn = st[e]
            out.append((e, jnp.where(odd_pair, up, ee),
                        pltpu.roll(jnp.where(odd_pair, up, a), 64, axis=1)))
            out.append((2 + e, jnp.where(odd_pair, ee, dn),
                        pltpu.roll(jnp.where(odd_pair, a, dn), 64, axis=1)))
        return out

    def kq3(i, g, z, st):
        r0 = pl.multiple_of(i * (TQ // 4) + z * (KQR // 4), KQR // 4)
        for j, own, oth in st:
            kh8[g * HG + j, pl.ds(r0, KQR // 4), :] = jnp.where(hi_half, oth, own)
            kh8[g * HG + 4 + j, pl.ds(r0, KQR // 4), :] = jnp.where(hi_half, own, oth)

    def ksplit_steps(i, invs, st, lo, hi, pace):
        for s in range(lo, hi):
            if s < nz:
                pr = (s - lo) * (pace.shape[0] // 8) // (hi - lo) * 8
                st[s] = kq0(i, s // zpg, s % zpg, _tie(invs[s // zpg], pace[pr:pr + 8]))
            if 0 <= s - 1 < nz:
                st[s - 1] = kq1(st[s - 1])
            if 0 <= s - 2 < nz:
                st[s - 2] = kq2(st[s - 2])
            if 0 <= s - 3 < nz:
                kq3(i, (s - 3) // zpg, (s - 3) % zpg, st.pop(s - 3))

    def vdot(i, n):
        xn = pltpu.bitcast(xn_s[i, n * 64:(n + 1) * 64, :], _BF)
        v = _nt_dot(pltpu.bitcast(wqvt[1], _BF), xn)
        vt[i, :, n * 128:(n + 1) * 128] = v
        return v

    def qdot(i, n):
        xn = pltpu.bitcast(xn_s[i, n * 64:(n + 1) * 64, :], _BF)
        qt_ = _nt_dot(pltpu.bitcast(wqvt[0], _BF), xn)
        ls = slice(n * 128, (n + 1) * 128)
        for h in range(H):
            q = qt_[h * DH:(h + 1) * DH]
            qm = jnp.maximum(jnp.max(jnp.abs(q), axis=0, keepdims=True), 1e-30)
            sq[i, h:h + 1, ls] = qm * qscale
            u = q * (127.0 * _recip(qm))
            ai = _rnd(u)
            bi = _rnd((u - ai.astype(_F32)) * float(NREP * 2 ** SC))
            asi = _rnd(u * (2.0 ** -SA))
            xx = [asi, bi] if h % 2 == 0 else [bi, asi]
            qw[i, h, :, ls] = _pack8(jnp.concatenate([ai, ai] + xx, axis=0))

    def phase1b(ii, carry):
        for u in range(P1U):
            i = ii * P1U + u
            invs = [kscale(i, g) for g in range(ng)]
            st = {}
            for n in range(nsub):
                ksplit_steps(i, invs, st, n * zpg, (n + 1) * zpg, vdot(i, n))
            ksplit_steps(i, invs, st, nz, nz + 3, None)
            for n in range(nsub):
                qdot(i, n)
        return carry

    lax.fori_loop(0, nt // P1U, phase1b, 0)
    for c in late_copies:
        c.wait()

    nf = S // KF
    fpt = TQ // KF
    bpt = ng // GP
    nstep = GP * HG * nf

    def fast_body(i, carry):
        lmax, lmin = carry
        qi = i // bpt
        h0 = (i % bpt) * (GP * HG)

        def scores(t):
            j, c = t // nf, t % nf
            w2 = qw[qi, h0 + j]
            aa, xx = w2[0:8], w2[8:16]
            w = jnp.concatenate([xx if r == (j % HG) // 2 else aa for r in range(4)], axis=0)
            kc = kh8[h0 + j, c * (KF // 4):(c + 1) * (KF // 4), :]
            return jnp.dot(pltpu.bitcast(kc, _I8), pltpu.bitcast(w, _I8),
                           preferred_element_type=_I32)

        pend = scores(0)
        l8 = acc = sqb = cs = None
        first = []
        for t in range(nstep):
            s = pend
            if t + 1 < nstep:
                pend = scores(t + 1)
            c = t % nf
            h = h0 + t // nf
            if c == 0:
                l8 = acc = None
                sqb = jnp.broadcast_to(sq[qi, pl.ds(h, 1), :], (8, TQ))
            if c % fpt == 0:
                cs = sqb * jnp.concatenate([skb[c // fpt, h]] * nsub, axis=1)
            p3 = jnp.exp2(s.astype(_F32).reshape(KF // 8, 8, TQ) * cs[None])
            for r in range(KF // 8):
                l8 = p3[r] if l8 is None else l8 + p3[r]
            p = jnp.concatenate([p3[b * 16 + r] for b in range(KF // 128)
                                 for r in range(15, -1, -1)], axis=0)
            v = vt[c // fpt, pl.ds(pl.multiple_of(h * DH, DH), DH), pl.ds((c % fpt) * KF, KF)]
            if t == nstep - 1:
                wr = pl.multiple_of(h0 * DH, 128)
                hres_s[qi] = _tn_dot(jnp.concatenate(first, axis=0),
                                     wo_v[pl.ds(wr, 128), :]) + hres_s[qi]
            pv = jnp.dot(v, p, preferred_element_type=_F32)
            acc = pv if acc is None else pv + acc
            if c == nf - 1:
                l = jnp.sum(l8, axis=0, keepdims=True)
                for z in range(nsub):
                    lz = l[:, z * 128:(z + 1) * 128]
                    lmax = jnp.maximum(lmax, lz)
                    lmin = jnp.minimum(lmin, lz)
                o = (acc * _recip(l)).astype(_BF)
                if t // nf < HG:
                    first.append(o)
                else:
                    ot[qi, pl.ds(pl.multiple_of(h * (DH // 2), DH // 2), DH // 2), :] = (
                        pltpu.bitcast(o, _U32))
        return lmax, lmin

    lmax, lmin = lax.fori_loop(
        0, nt * bpt, fast_body, (jnp.ones((1, 128), _F32), jnp.ones((1, 128), _F32)))

    def fast_path_unsafe():
        sqm = jnp.max(jnp.max(sq[...], axis=0), axis=1, keepdims=True)
        skm = jnp.max(skb[:, :, 0, :], axis=0)
        cmax = jnp.max(sqm * skm, axis=0, keepdims=True)
        ok = ((cmax <= CMAX / (NREP * 127.0 * 127.0)) & (lmax <= LMAX) & (lmin >= 1.0 / LMAX))
        return jnp.sum(jnp.where(ok, 1.0, 0.0)) < 128.0

    def wo_part(i, par):
        gs = range(par, ng, GP)
        o_t = jnp.concatenate([ot[i, g * 64:(g + 1) * 64, :] for g in gs], axis=0)
        w = jnp.concatenate([wo_v[g * 128:(g + 1) * 128, :] for g in gs], axis=0)
        return _tn_dot(pltpu.bitcast(o_t, _BF), w)

    def slow_attention():
        cpt = TQ // KC

        def prep(z, carry):
            r2 = pl.multiple_of((z % nsub) * 64, 64)
            xn = pltpu.bitcast(xn_s[z // nsub, pl.ds(r2, 64), :], _BF)
            kf = jnp.dot(xn, wqkv_v[1], preferred_element_type=_F32)
            ku = pltpu.bitcast(kf.astype(_BF), _U32)
            rh = pl.multiple_of(z * 64, 64)
            for g in range(ng):
                kg = ku[:, g * 128:(g + 1) * 128]
                for j in range(HG):
                    kr = kg if j == 0 else pltpu.roll(kg, 128 - DH * j, axis=1)
                    kh[g * HG + j, pl.ds(rh, 64), :] = kr
            q = _nt_dot(pltpu.bitcast(wqvt[0], _BF), xn)
            qt[z] = pltpu.bitcast((q * qscale).astype(_BF), _U32)
            return carry

        lax.fori_loop(0, nt * nsub, prep, 0)

        def item(it, carry):
            h = it % H
            qi = it // H
            hr = pl.multiple_of(h * (DH // 2), DH // 2)
            q = pltpu.bitcast(jnp.concatenate(
                [qt[qi * nsub + n, pl.ds(hr, DH // 2), :] for n in range(nsub)], axis=1), _BF)

            def pass1(c, m8):
                kr = pl.multiple_of(c * (KC // 2), KC // 2)
                kc = pltpu.bitcast(kh[h, pl.ds(kr, KC // 2), :], _BF)[:, :DH]
                s = jnp.dot(kc, q, preferred_element_type=_F32)
                sbuf[c] = s
                return jnp.maximum(m8, jnp.max(s.reshape(KC // 8, 8, TQ), axis=0))

            m8 = lax.fori_loop(0, S // KC, pass1, jnp.full((8, TQ), -jnp.inf, _F32))
            m = jnp.max(m8, axis=0, keepdims=True)

            def pass2(ti, la):
                l8, acc = la
                for cc in range(cpt):
                    p = jnp.exp2(sbuf[ti * cpt + cc] - m)
                    l8 = l8 + jnp.sum(p.reshape(KC // 8, 8, TQ), axis=0)
                    v = vt[ti, pl.ds(pl.multiple_of(h * DH, DH), DH), cc * KC:(cc + 1) * KC]
                    acc = acc + jnp.dot(v, p, preferred_element_type=_F32)
                return l8, acc

            l8, acc = lax.fori_loop(0, nt, pass2,
                                    (jnp.zeros((8, TQ), _F32), jnp.zeros((DH, TQ), _F32)))
            o = acc * (1.0 / jnp.sum(l8, axis=0, keepdims=True))
            ot[qi, pl.ds(hr, DH // 2), :] = pltpu.bitcast(o.astype(_BF), _U32)
            return carry

        lax.fori_loop(0, nt * H, item, 0)

        def redo(i, carry):
            r0 = pl.multiple_of(i * TQ, TQ)
            hres_s[i] = x_v[pl.ds(r0, TQ), :].astype(_F32) + wo_part(i, 0)
            return carry

        lax.fori_loop(0, nt, redo, 0)

    def ln2(i, pace):
        for n in range(nsub):
            hn = _layernorm(hres_s[i, n * 128:(n + 1) * 128, :], _pace_rows(pace, n, nsub))
            hn_s[0, n * 64:(n + 1) * 64, :] = pltpu.bitcast(hn.astype(_BF), _U32)

    def wo_stage(c):
        pl.when(c[0] == 1)(slow_attention)
        pace = []
        for i in range(nt):
            hres = wo_part(i, 1) + hres_s[i]
            hres_s[i] = hres
            if i in (1, 2):
                pace.append(jnp.concatenate([hres[:, 0:128], hres[:, D - 128:D]], axis=0))
        ln2(0, jnp.concatenate(pace, axis=0))
        return c[0] + 1, jnp.where(fast_path_unsafe(), 2, 1).astype(_I32)

    lax.while_loop(lambda c: c[0] < c[1], wo_stage, (jnp.int32(0), jnp.int32(1)))

    orows = TQ // OSPLIT

    def out_copy(i, k):
        r0 = pl.multiple_of(i * TQ + k * orows, orows)
        return pltpu.make_async_copy(obuf.at[pl.ds(r0, orows)], out_hbm.at[pl.ds(r0, orows)],
                                     sem_out.at[0])

    def ffn(i, carry):
        hn_u = hn_s[0]
        hn_s[1] = hn_u
        acc = hres_s[i] + b2_v[...].astype(_F32)[None, :]
        for f0 in range(0, F, FC):
            hn = pltpu.bitcast(hn_u if f0 == 0 else hn_s[1], _BF)
            z = jnp.dot(hn, w1_v[:, f0:f0 + FC], preferred_element_type=_F32)
            z = _gelu(z + b1_v[f0:f0 + FC].astype(_F32)[None, :]).astype(_BF)
            if f0 + FC < F:
                acc = jnp.dot(z, w2_v[f0:f0 + FC, :], preferred_element_type=_F32) + acc
                if f0 == 0:
                    ln2(jnp.minimum(i + 1, nt - 1),
                        jnp.concatenate([acc[:, 0:128], acc[:, D - 128:D]], axis=0))
            else:
                for k in range(OSPLIT):
                    rs = slice(k * orows, (k + 1) * orows)
                    o = jnp.dot(z[rs], w2_v[f0:f0 + FC, :], preferred_element_type=_F32) + acc[rs]
                    r0 = pl.multiple_of(i * TQ + k * orows, orows)
                    obuf[pl.ds(r0, orows), :] = o.astype(obuf.dtype)
                    out_copy(i, k).start()
        return carry

    lax.fori_loop(0, nt, ffn, 0)
    for i in range(nt):
        for k in range(OSPLIT):
            out_copy(i, k).wait()


@jax.jit
def pallas_sequential_preLN__softmax_full_mha__dense_activation_gelu__prompt_kernel(
    A_x: jax.Array,
    A_wqkv: jax.Array,
    A_wo: jax.Array,
    B_x: jax.Array,
    B_w1: jax.Array,
    B_b1: jax.Array,
    B_w2: jax.Array,
    B_b2: jax.Array,
):
    del B_x
    B, S, D = A_x.shape
    F = B_w1.shape[1]
    assert B == 1 and D == H * DH
    nt = S // TQ
    any_spec = pl.BlockSpec(memory_space=pl.ANY)
    out = pl.pallas_call(
        functools.partial(_kernel, S=S, D=D, F=F),
        out_shape=jax.ShapeDtypeStruct((S, D), A_x.dtype),
        in_specs=[any_spec] * 7,
        out_specs=any_spec,
        scratch_shapes=[
            pltpu.VMEM((F,), _BF),
            pltpu.VMEM((D,), _BF),
            pltpu.VMEM((S, D), _BF),
            pltpu.VMEM((3, D, D), _BF),
            pltpu.VMEM((D, D), _BF),
            pltpu.VMEM((D, F), _BF),
            pltpu.VMEM((F, D), _BF),
            pltpu.VMEM((2, D // 2, D), _U32),
            pltpu.VMEM((nt, TQ // 2, D), _U32),
            pltpu.VMEM((nt, D // 128, TQ, 128), _F32),
            pltpu.VMEM((nt, D // 128, 8, 128), _F32),
            pltpu.VMEM((H, S // 4, 128), _U32),
            pltpu.VMEM((nt, H, 16, TQ), _U32),
            pltpu.VMEM((nt, H, TQ), _F32),
            pltpu.VMEM((nt, H, 8, 128), _F32),
            pltpu.VMEM((nt, D, TQ), _F32),
            pltpu.VMEM((nt, D // 2, TQ), _U32),
            pltpu.VMEM((2, TQ // 2, D), _U32),
            pltpu.VMEM((nt, TQ, D), _F32),
            pltpu.VMEM((S, D), _BF),
            pltpu.VMEM((H, S // 2, 128), _U32),
            pltpu.VMEM((S // 128, D // 2, 128), _U32),
            pltpu.VMEM((S // KC, KC, TQ), _F32),
            pltpu.SemaphoreType.DMA((nt + 4,)),
            pltpu.SemaphoreType.DMA((1,)),
        ],
        compiler_params=pltpu.CompilerParams(vmem_limit_bytes=110 * 1024 * 1024),
    )(A_x.reshape(S, D), A_wqkv, A_wo, B_w1, B_w2, B_b1, B_b2)
    return out.reshape(B, S, D)
```
